```python
import os as _os
_os.environ.setdefault('JAX_PLATFORMS', 'cpu')
import jax
import jax.numpy as jnp

def _softmax(x, axis=-1):
    return jax.nn.softmax(x, axis=axis)

def _gelu(x):
    return jax.nn.gelu(x, approximate=True)

def _silu(x):
    return jax.nn.silu(x)

def _sigmoid(x):
    return jax.nn.sigmoid(x)

def _layernorm(x, axis=-1, eps=1e-05):
    m = jnp.mean(x, axis=axis, keepdims=True)
    v = jnp.var(x, axis=axis, keepdims=True)
    return (x - m) / jnp.sqrt(v + eps)

def _scatter_add(tgt, idx, src, axis=0):
    return tgt.at[idx].add(src)

def _segment_sum(src, seg, n):
    return jax.ops.segment_sum(src, seg, n)

class _Rng:

    def __init__(self, key):
        self._k = key

    def _next(self):
        self._k, sub = jax.random.split(self._k)
        return sub

    def normal(self, shape):
        return jax.random.normal(self._next(), shape, dtype=jnp.bfloat16)

    def randint(self, lo, hi, shape):
        return jax.random.randint(self._next(), shape, lo, hi, dtype=jnp.int32)

    def uniform(self, shape, lo=0.0, hi=1.0):
        return jax.random.uniform(self._next(), shape, jnp.bfloat16, lo, hi)

    def permutation(self, n):
        return jax.random.permutation(self._next(), n)
kernel_name = 'sequential_preLN__memory_aug_recurrent_mem_tr__swiglu_ffn__prompt'

def setup_inputs():
    _rng = _Rng(jax.random.key(int.from_bytes(__import__("os").urandom(4), "little")))
    _w = lambda a: (lambda t: t.astype(jnp.bfloat16) if jnp.issubdtype(t.dtype, jnp.floating) else t)(jnp.asarray(a))

    def _A_setup():
        B, S, Dm = (1, 2048, 640)
        H, Dh = (32, 192)
        M, seg = (8, 32)
        seg = min(seg, S)
        S = S // seg * seg
        return {'x': _w((lambda *s: _rng.normal(s) * 0.05)(B, S, Dm)), 'mem0': _w((lambda *s: _rng.normal(s) * 0.1)(B, M, Dm)), 'Wq': _w((lambda *s: _rng.normal(s) * 1.6)(Dm, H, Dh) * Dm ** (-0.5)), 'Wk': _w((lambda *s: _rng.normal(s) * 1.6)(Dm, H, Dh) * Dm ** (-0.5)), 'Wv': _w((lambda *s: _rng.normal(s) * 0.1)(Dm, H, Dh) * Dm ** (-0.5)), 'Wo': _w((lambda *s: _rng.normal(s) * 0.1)(H, Dh, Dm) * (H * Dh) ** (-0.5)), 'seg_len': seg}
    _A_in = _A_setup()

    def _B_setup():
        B, S, D, F = (1, 2048, 640, 1536)
        return {'x': _w((lambda *s: _rng.normal(s) * 0.05)(B, S, D)), 'w_gate': _w((lambda *s: _rng.normal(s) * 0.05)(D, F)), 'w_up': _w((lambda *s: _rng.normal(s) * 0.05)(D, F)), 'w_down': _w((lambda *s: _rng.normal(s) * 0.05)(F, D))}
    _B_in = _B_setup()
    return {'A_x': _A_in['x'], 'A_mem0': _A_in['mem0'], 'A_Wq': _A_in['Wq'], 'A_Wk': _A_in['Wk'], 'A_Wv': _A_in['Wv'], 'A_Wo': _A_in['Wo'], 'A_seg_len': _A_in['seg_len'], 'B_x': _B_in['x'], 'B_w_gate': _B_in['w_gate'], 'B_w_up': _B_in['w_up'], 'B_w_down': _B_in['w_down']}

def reference(A_x, A_mem0, A_Wq, A_Wk, A_Wv, A_Wo, A_seg_len, B_x, B_w_gate, B_w_up, B_w_down):

    def _A_ref(x, mem0, Wq, Wk, Wv, Wo, seg_len):
        B, S, Dm = x.shape
        H, Dh = (Wq.shape[1], Wq.shape[2])
        M = mem0.shape[1]
        scale = Dh ** (-0.5)
        n_seg = S // seg_len
        L = M + seg_len
        idx = jnp.arange(L)
        mask = (idx[:, None] < M) | (idx[:, None] >= idx[None, :])
        mem = mem0
        outs = []
        for s in range(n_seg):
            xs = x[:, s * seg_len:(s + 1) * seg_len, :].copy()
            h = jnp.concatenate([mem, xs], axis=1)
            q = jnp.einsum('btd,dhe->bhte', h, Wq)
            k = jnp.einsum('btd,dhe->bhte', h, Wk)
            v = jnp.einsum('btd,dhe->bhte', h, Wv)
            scores = jnp.einsum('bhqe,bhke->bhqk', q, k) * scale
            scores = jnp.where(mask[None, None], scores, -1000000000.0)
            p = _softmax(scores, axis=-1)
            o = jnp.einsum('bhqk,bhke->bhqe', p, v)
            o = jnp.einsum('bhte,hed->btd', o, Wo)
            mem = o[:, :M, :].copy()
            outs.append(o[:, M:, :])
        return jnp.concatenate(outs, axis=1)

    def _B_ref(x, w_gate, w_up, w_down):
        g = _silu(x @ w_gate)
        u = x @ w_up
        return g * u @ w_down
    x = A_x
    h = x + _A_ref(_layernorm(x, axis=-1), A_mem0, A_Wq, A_Wk, A_Wv, A_Wo, A_seg_len)
    h2 = h + _B_ref(_layernorm(h, axis=-1), B_w_gate, B_w_up, B_w_down)
    return h2
```

```python
import functools
import jax
import jax.numpy as jnp
from jax import lax
import jax.experimental.pallas as pl
import jax.experimental.pallas.tpu as pltpu

S = 2048
D = 640
H = 32
DH = 192
HD = H * DH
M = 8
SEG = 32
NSEG = S // SEG
F = 1536
EPS = 1e-5
RIDE = 24
PRO = S - RIDE * NSEG
RING = 576
CH = 512
NCH = HD // CH
NBUF = 3
FCH = 256
KP = 48

bf16 = jnp.bfloat16
f32 = jnp.float32
u32 = jnp.uint32


def _ln(x):
    m = jnp.mean(x, axis=-1, keepdims=True)
    xc = x - m
    v = jnp.mean(xc * xc, axis=-1, keepdims=True)
    return xc * lax.rsqrt(v + EPS)


def _as_bf16(w32):
    return pltpu.bitcast(w32, bf16)


def _kernel(x_hbm, mem0_ref, wq_hbm, wk_hbm, wv_hbm, wo_hbm, wg_hbm, wu_hbm, wd_hbm,
            out_hbm,
            x_v, xn_pro, stage, wqkv, wo_raw, wo32, wg_v, wu_v, wd_v,
            ring, oring, h_v, mem_v, ostage,
            sem_x, sem_stage, sem_wo, sem_ffn, sem_out):
    w_hbms = (wq_hbm, wk_hbm, wv_hbm)

    def x_copy(i):
        if i == 0:
            return pltpu.make_async_copy(x_hbm.at[pl.ds(0, PRO)], x_v.at[pl.ds(0, PRO)], sem_x.at[0])
        return pltpu.make_async_copy(x_hbm.at[pl.ds(PRO, S - PRO)], x_v.at[pl.ds(PRO, S - PRO)], sem_x.at[1])

    def w_copy(mat, c, slot):
        return pltpu.make_async_copy(
            w_hbms[mat].at[pl.ds(pl.multiple_of(c * CH, CH), CH)], stage.at[slot], sem_stage.at[slot])

    def wo_copy():
        return pltpu.make_async_copy(wo_hbm, wo_raw, sem_wo.at[0])

    def ffn_copy(i):
        src, dst = ((wg_hbm, wg_v), (wu_hbm, wu_v), (wd_hbm, wd_v))[i]
        return pltpu.make_async_copy(src, dst, sem_ffn.at[i])

    x_copy(0).start()
    for b in range(NBUF):
        w_copy(0, b, b).start()
    x_copy(0).wait()
    xn_pro[...] = _ln(x_v[pl.ds(0, PRO), :].astype(f32)).astype(bf16)
    mem_v[...] = mem0_ref[...].astype(f32)
    oring[pl.ds(0, RIDE), :] = jnp.zeros((RIDE, HD), f32)

    for mat in range(3):
        def pro_body(c, carry, mat=mat):
            g = mat * NCH + c
            slot = g % NBUF
            w_copy(mat, c, slot).wait()
            blk = stage[slot]
            t = blk.T
            col = pl.multiple_of(g * CH, CH)
            wqkv[:, pl.ds(col, CH)] = pltpu.bitcast(t, u32)
            y = lax.dot_general(xn_pro[...], blk, (((1,), (1,)), ((), ())), preferred_element_type=f32)
            ring[pl.ds(RING - PRO, PRO), pl.ds(col, CH)] = y.astype(bf16)

            @pl.when(c + NBUF < NCH)
            def _():
                w_copy(mat, c + NBUF, slot).start()
            if mat < 2:
                @pl.when(c + NBUF >= NCH)
                def _():
                    w_copy(mat + 1, c + NBUF - NCH, slot).start()
            return carry
        if mat == 1:
            wo_copy().start()
        if mat == 2:
            x_copy(1).start()
            for i in range(3):
                ffn_copy(i).start()
        lax.fori_loop(0, NCH, pro_body, 0)

    wo_copy().wait()

    def wo_conv(c, carry):
        r = pl.multiple_of(c * CH, CH)
        r2 = pl.multiple_of(c * (CH // 2), CH // 2)
        wo32[pl.ds(r2, CH // 2), :] = pltpu.bitcast(wo_raw[pl.ds(r, CH), :], u32)
        return carry
    lax.fori_loop(0, NCH, wo_conv, 0)
    x_copy(1).wait()

    scale = DH ** (-0.5)
    lane = lax.broadcasted_iota(jnp.int32, (40, 2 * KP), 1)
    row = lax.broadcasted_iota(jnp.int32, (40, 2 * KP), 0)
    isA = lane < KP
    kidx = jnp.where(isA, lane, lane - KP)
    real = kidx < SEG + M
    visible = (row >= SEG) | (kidx >= SEG) | (kidx <= row)
    lo128 = lax.broadcasted_iota(jnp.int32, (KP // 2, 128), 1) < 64
    zeros_t = jnp.zeros((KP // 2, 128), u32)

    def blockdiag(a48):
        a32 = pltpu.bitcast(a48, u32)
        t0, t1, t2 = a32[:, 0:128], a32[:, 128:256], a32[:, 256:384]
        top = jnp.concatenate([t0, jnp.where(lo128, t1, jnp.uint32(0)), zeros_t], axis=1)
        bot = jnp.concatenate([zeros_t, jnp.where(lo128, jnp.uint32(0), t1), t2], axis=1)
        return pltpu.bitcast(jnp.concatenate([top, bot], axis=0), bf16)

    def step(s, carry):
        xr = pl.multiple_of(PRO + RIDE * s, 8)
        xn = _ln(x_v[pl.ds(xr, RIDE), :].astype(f32))
        lhs = jnp.concatenate([xn, mem_v[...]], axis=0).astype(bf16)
        wslot = pl.multiple_of((RIDE * s) % RING, 8)
        rslot = pl.multiple_of((SEG * s + RING - PRO) % RING, 32)
        owslot = pl.multiple_of((SEG * s) % RING, 32)
        otok = RIDE * jnp.maximum(s - 1, 0)
        orslot = pl.multiple_of(otok % RING, 8)
        zpad = jnp.zeros((8, 384), f32)
        NP = H // 2

        def proj(p):
            c0 = p * 384
            parts = []
            for mat in range(3):
                col = mat * HD + c0
                y = jnp.dot(lhs, _as_bf16(wqkv[:, col:col + 384]), preferred_element_type=f32)
                ring[pl.ds(wslot, RIDE), col:col + 384] = y[:RIDE].astype(bf16)
                parts.append(jnp.concatenate([y[RIDE:], zpad], axis=0).astype(bf16))
            return parts

        def tok(mat, p):
            col = mat * HD + p * 384
            return ring[pl.ds(rslot, SEG), col:col + 384]

        def scores(qt, kt, qm, km):
            q48 = jnp.concatenate([qt, qm], axis=0)
            kbd = blockdiag(jnp.concatenate([kt, km], axis=0))
            sc = lax.dot_general(q48, kbd, (((1,), (1,)), ((), ())), preferred_element_type=f32)
            sc = sc[:40] * scale
            sc = jnp.where(visible, sc, -1e9)
            sc = jnp.where(real, sc, -jnp.inf)
            mA = jnp.max(jnp.where(isA, sc, -jnp.inf), axis=-1, keepdims=True)
            mB = jnp.max(jnp.where(isA, -jnp.inf, sc), axis=-1, keepdims=True)
            e = jnp.exp(sc - jnp.where(isA, mA, mB))
            lA = jnp.sum(jnp.where(isA, e, 0.0), axis=-1, keepdims=True)
            lB = jnp.sum(jnp.where(isA, 0.0, e), axis=-1, keepdims=True)
            pr = e / jnp.where(isA, lA, lB)
            return jnp.concatenate([pr, jnp.zeros((8, 2 * KP), f32)], axis=0).astype(bf16)

        def pv(p, pr, vt, vm):
            c0 = p * 384
            vbd = blockdiag(jnp.concatenate([vt, vm], axis=0))
            o = jnp.dot(pr, vbd, preferred_element_type=f32)
            oring[pl.ds(owslot, SEG), c0:c0 + 384] = o[:SEG]
            return o[SEG:SEG + M]

        def wo(p, ot, om):
            c0 = p * 384
            lhs2 = jnp.concatenate([ot, om], axis=0).astype(bf16)
            return jnp.dot(lhs2, _as_bf16(wo32[c0 // 2:c0 // 2 + 192, :]), preferred_element_type=f32)

        acc = None
        pm, prs, oms = {}, {}, {}
        for i in range(NP + 3):
            if 0 <= i - 1 < NP:
                qt, kt = tok(0, i - 1), tok(1, i - 1)
            if 0 <= i - 2 < NP:
                vt = tok(2, i - 2)
            if 0 <= i - 3 < NP:
                ot = oring[pl.ds(orslot, RIDE), (i - 3) * 384:(i - 2) * 384]
            if i < NP:
                pm[i] = proj(i)
            if 0 <= i - 1 < NP:
                prs[i - 1] = scores(qt, kt, pm[i - 1][0], pm[i - 1][1])
            if 0 <= i - 2 < NP:
                oms[i - 2] = pv(i - 2, prs.pop(i - 2), vt, pm.pop(i - 2)[2])
            if 0 <= i - 3 < NP:
                w = wo(i - 3, ot, oms.pop(i - 3))
                acc = w if acc is None else acc + w
        hr = pl.multiple_of(otok, 8)
        h_v[pl.ds(hr, RIDE), :] = x_v[pl.ds(hr, RIDE), :].astype(f32) + acc[:RIDE]
        mem_v[...] = acc[RIDE:].astype(bf16).astype(f32)
        return carry

    lax.fori_loop(0, NSEG, step, 0)

    t0 = RIDE * (NSEG - 1)
    s0 = t0 % RING
    n1 = RING - s0
    for (slot, tok, n) in ((s0, t0, n1), (0, t0 + n1, S - t0 - n1)):
        a = jnp.dot(oring[pl.ds(slot, n), :].astype(bf16), _as_bf16(wo32[...]), preferred_element_type=f32)
        h_v[pl.ds(tok, n), :] = x_v[pl.ds(tok, n), :].astype(f32) + a

    for i in range(3):
        ffn_copy(i).wait()

    def out_copy(c, slot):
        return pltpu.make_async_copy(ostage.at[slot], out_hbm.at[pl.ds(pl.multiple_of(c * FCH, FCH), FCH)],
                                     sem_out.at[slot])

    def ffn_body(c, carry):
        r = pl.multiple_of(c * FCH, FCH)
        slot = c % 2
        h = h_v[pl.ds(r, FCH), :].astype(bf16).astype(f32)
        hn = _ln(h).astype(bf16)
        acc = h
        for f0 in range(0, F, 512):
            g = jnp.dot(hn, wg_v[:, f0:f0 + 512], preferred_element_type=f32)
            u = jnp.dot(hn, wu_v[:, f0:f0 + 512], preferred_element_type=f32)
            a = (g * jax.nn.sigmoid(g) * u).astype(bf16)
            acc = acc + jnp.dot(a, wd_v[f0:f0 + 512, :], preferred_element_type=f32)

        @pl.when(c >= 2)
        def _():
            out_copy(c - 2, slot).wait()
        ostage[slot] = acc.astype(bf16)
        out_copy(c, slot).start()
        return carry

    nfc = S // FCH
    lax.fori_loop(0, nfc, ffn_body, 0)
    out_copy(nfc - 2, (nfc - 2) % 2).wait()
    out_copy(nfc - 1, (nfc - 1) % 2).wait()


@jax.jit
def pallas_sequential_preLN__memory_aug_recurrent_mem_tr__swiglu_ffn__prompt_kernel(A_x, A_mem0, A_Wq, A_Wk, A_Wv, A_Wo, A_seg_len, B_x, B_w_gate, B_w_up, B_w_down):
    del A_seg_len, B_x
    x = A_x.reshape(S, D)
    mem0 = A_mem0.reshape(M, D)
    wqt = jnp.transpose(A_Wq, (1, 2, 0)).reshape(HD, D)
    wkt = jnp.transpose(A_Wk, (1, 2, 0)).reshape(HD, D)
    wvt = jnp.transpose(A_Wv, (1, 2, 0)).reshape(HD, D)
    wo = A_Wo.reshape(HD, D)
    any_spec = pl.BlockSpec(memory_space=pl.ANY)
    out = pl.pallas_call(
        _kernel,
        out_shape=jax.ShapeDtypeStruct((S, D), bf16),
        in_specs=[any_spec, pl.BlockSpec(memory_space=pltpu.VMEM)] + [any_spec] * 7,
        out_specs=any_spec,
        scratch_shapes=[
            pltpu.VMEM((S, D), bf16),
            pltpu.VMEM((PRO, D), bf16),
            pltpu.VMEM((NBUF, CH, D), bf16),
            pltpu.VMEM((D // 2, 3 * HD), u32),
            pltpu.VMEM((HD, D), bf16),
            pltpu.VMEM((HD // 2, D), u32),
            pltpu.VMEM((D, F), bf16),
            pltpu.VMEM((D, F), bf16),
            pltpu.VMEM((F, D), bf16),
            pltpu.VMEM((RING, 3 * HD), bf16),
            pltpu.VMEM((RING, HD), f32),
            pltpu.VMEM((S, D), f32),
            pltpu.VMEM((M, D), f32),
            pltpu.VMEM((2, FCH, D), bf16),
            pltpu.SemaphoreType.DMA((2,)),
            pltpu.SemaphoreType.DMA((NBUF,)),
            pltpu.SemaphoreType.DMA((1,)),
            pltpu.SemaphoreType.DMA((3,)),
            pltpu.SemaphoreType.DMA((2,)),
        ],
        compiler_params=pltpu.CompilerParams(vmem_limit_bytes=120 * 1024 * 1024),
    )(x, mem0, wqt, wkt, wvt, wo, B_w_gate, B_w_up, B_w_down)
    return out.reshape(1, S, D)
```

```python
import functools
import os
import jax
import jax.numpy as jnp
from jax import lax
import jax.experimental.pallas as pl
import jax.experimental.pallas.tpu as pltpu

S = 2048
D = 640
H = 32
DH = 192
HD = H * DH
M = 8
SEG = 32
NSEG = S // SEG
F = 1536
EPS = 1e-5
RIDE = 24
PRO = S - RIDE * NSEG
RING = 576
CH = 1024
NCH = HD // CH
NBUF = 3
KP = 48
NP = H // 2
PW = 2 * DH
FB = 2 * SEG
NFS = 2
FC = F // NFS
WO_LAG = int(os.environ.get('WO_LAG', 7))

bf16 = jnp.bfloat16
f32 = jnp.float32
u32 = jnp.uint32


def _ln(x):
    m = jnp.mean(x, axis=-1, keepdims=True)
    xc = x - m
    v = jnp.mean(xc * xc, axis=-1, keepdims=True)
    return xc * lax.rsqrt(v + EPS)


def _as_bf16(w32):
    return pltpu.bitcast(w32, bf16)


def _step_order():
    order = []
    for i in range(NP):
        order.append(('qk', i))
        if i >= 1:
            order.append(('v', i - 1))
            order.append(('s', i - 1))
        if i >= 3:
            order.append(('pv', i - 3))
        if i >= WO_LAG:
            order.append(('wo', i - WO_LAG))
    rem = list(range(NP - WO_LAG, NP))
    tail = [('v', 15), ('pv', 13), ('wo', None), ('s', 15), ('wo', None), ('pv', 14), ('wo', None),
            ('wo', None), ('wo', None), ('pv', 15), ('wo', None), ('wo', None)]
    for op, p in tail:
        if op == 'wo':
            if rem:
                order.append(('wo', rem.pop(0)))
        else:
            order.append((op, p))
    for p in rem:
        order.append(('wo', p))
    return order


def _kernel(x_hbm, mem0_ref, wq_hbm, wk_hbm, wv_hbm, wo_hbm, wg_hbm, wu_hbm, wd_hbm,
            out_hbm,
            x_v, xn_v, stage, wqkv, wo_raw, wo32, wg_v, wu_v, wd_v,
            ring, h_v, mem_v, out_v,
            sem_x, sem_stage, sem_wo, sem_ffn, sem_out):
    w_hbms = (wq_hbm, wk_hbm, wv_hbm)

    def x_copy(i):
        r = pl.multiple_of(i * PRO, PRO)
        return pltpu.make_async_copy(x_hbm.at[pl.ds(r, PRO)], x_v.at[pl.ds(r, PRO)], sem_x.at[i])

    def w_copy(mat, c, slot):
        return pltpu.make_async_copy(
            w_hbms[mat].at[pl.ds(pl.multiple_of(c * CH, CH), CH)], stage.at[slot], sem_stage.at[slot])

    def wo_copy(c):
        r = pl.multiple_of(c * CH, CH)
        return pltpu.make_async_copy(wo_hbm.at[pl.ds(r, CH)], wo_raw.at[pl.ds(r, CH)], sem_wo.at[c])

    def ffn_copy(i):
        src, dst = ((wg_hbm, wg_v), (wu_hbm, wu_v), (wd_hbm, wd_v))[i]
        return pltpu.make_async_copy(src, dst, sem_ffn.at[i])

    def out_copy(r, n):
        return pltpu.make_async_copy(out_v.at[pl.ds(r, n)], out_hbm.at[pl.ds(r, n)], sem_out.at[0])

    x_copy(0).start()
    for b in range(NBUF):
        w_copy(0, b, b).start()
    mem_v[...] = mem0_ref[...].astype(f32)
    h_v[...] = jnp.zeros((FB, D), f32)
    x_copy(0).wait()
    xn_v[pl.ds(0, PRO), :] = _ln(x_v[pl.ds(0, PRO), :].astype(f32)).astype(bf16)

    LNR = (S - PRO) // NCH

    for mat in range(3):
        def pro_body(c, carry, mat=mat):
            g = mat * NCH + c
            slot = g % NBUF
            w_copy(mat, c, slot).wait()
            if mat == 2:
                wo_copy(c).wait()
            blk = stage[slot]
            col = pl.multiple_of(g * CH, CH)
            y = lax.dot_general(xn_v[pl.ds(0, PRO), :], blk, (((1,), (1,)), ((), ())), preferred_element_type=f32)
            ring[pl.ds(RING - PRO, PRO), pl.ds(col, CH)] = y.astype(bf16)
            wqkv[:, pl.ds(col, CH)] = pltpu.bitcast(blk.T, u32)
            if mat == 1:
                r = pl.multiple_of(PRO + c * LNR, LNR)
                xn_v[pl.ds(r, LNR), :] = _ln(x_v[pl.ds(r, LNR), :].astype(f32)).astype(bf16)
            if mat == 2:
                r = pl.multiple_of(c * CH, CH)
                r2 = pl.multiple_of(c * (CH // 2), CH // 2)
                wo32[pl.ds(r2, CH // 2), :] = pltpu.bitcast(wo_raw[pl.ds(r, CH), :], u32)

            @pl.when(c + NBUF < NCH)
            def _():
                w_copy(mat, c + NBUF, slot).start()
            if mat < 2:
                @pl.when(c + NBUF >= NCH)
                def _():
                    w_copy(mat + 1, c + NBUF - NCH, slot).start()
            if mat == 0:
                @pl.when(c < 3)
                def _():
                    x_copy(c + 1).start()

                @pl.when(c >= 3)
                def _():
                    wo_copy(c - 3).start()
            if mat == 1:
                @pl.when(c < 3)
                def _():
                    wo_copy(c + NCH - 3).start()
            if mat == 2:
                for i in range(3):
                    @pl.when(c == NCH - 4 + i)
                    def _(i=i):
                        ffn_copy(i).start()
            return carry
        if mat == 1:
            for i in range(1, 4):
                x_copy(i).wait()
        lax.fori_loop(0, NCH, pro_body, 0)

    for i in range(3):
        ffn_copy(i).wait()

    scale = DH ** (-0.5)
    NK = 2 * (SEG + M)
    lane = lax.broadcasted_iota(jnp.int32, (40, NK), 1)
    row = lax.broadcasted_iota(jnp.int32, (40, NK), 0)
    isA = lane < SEG + M
    tokidx = jnp.where(isA, lane, lane - (SEG + 2 * M))
    is_mem_key = (lane >= SEG) & (lane < SEG + 2 * M)
    visible = (row >= SEG) | is_mem_key | (tokidx <= row)
    lo16 = lax.broadcasted_iota(jnp.int32, (SEG // 2, 128), 1) < 64
    lo8 = lax.broadcasted_iota(jnp.int32, (M, 128), 1) < 64
    lo40 = lax.broadcasted_iota(jnp.int32, (SEG + M, 128), 1) < 64
    z16 = jnp.zeros((SEG // 2, 128), u32)
    z8 = jnp.zeros((M, 128), f32)
    order = _step_order()

    def blockdiag(t, m):
        t32 = pltpu.bitcast(t, u32)
        t0, t1, t2 = t32[:, 0:128], t32[:, 128:256], t32[:, 256:384]
        top = jnp.concatenate([t0, jnp.where(lo16, t1, jnp.uint32(0)), z16], axis=1)
        bot = jnp.concatenate([z16, jnp.where(lo16, jnp.uint32(0), t1), t2], axis=1)
        m0, m1, m2 = m[:, 0:128], m[:, 128:256], m[:, 256:384]
        ma = jnp.concatenate([m0, jnp.where(lo8, m1, 0.0), z8], axis=1)
        mb = jnp.concatenate([z8, jnp.where(lo8, 0.0, m1), m2], axis=1)
        mid = pltpu.bitcast(jnp.concatenate([ma, mb], axis=0).astype(bf16), u32)
        return pltpu.bitcast(jnp.concatenate([top, mid, bot], axis=0), bf16)

    def segment(s, mem, carry_o, extra):
        xr = pl.multiple_of(PRO + RIDE * s, 8)
        xn = xn_v[pl.ds(xr, RIDE), :].astype(f32)
        lhs = jnp.concatenate([xn, mem], axis=0).astype(bf16)
        wslot = pl.multiple_of((RIDE * s) % RING, 8)
        rslot = pl.multiple_of((SEG * s + RING - PRO) % RING, 32)
        zpad = jnp.zeros((8, PW), f32)
        handed = {}

        def proj(mat, p):
            col = mat * HD + p * PW
            y = jnp.dot(lhs, _as_bf16(wqkv[:, col:col + PW]), preferred_element_type=f32)
            ring[pl.ds(wslot, RIDE), col:col + PW] = y[:RIDE].astype(bf16)
            return y[RIDE:]

        def tok(mat, p):
            col = mat * HD + p * PW
            return ring[pl.ds(rslot, SEG), col:col + PW]

        def scores(qt, kt, qm, km):
            q48 = jnp.concatenate([qt, jnp.concatenate([qm, zpad], axis=0).astype(bf16)], axis=0)
            kbd = blockdiag(kt, km)
            sc = lax.dot_general(q48, kbd, (((1,), (1,)), ((), ())), preferred_element_type=f32)
            sc = sc[:40] * scale
            sc = jnp.where(visible, sc, -1e9)
            mA = jnp.max(jnp.where(isA, sc, -jnp.inf), axis=-1, keepdims=True)
            mB = jnp.max(jnp.where(isA, -jnp.inf, sc), axis=-1, keepdims=True)
            e = jnp.exp(sc - jnp.where(isA, mA, mB))
            lA = jnp.sum(jnp.where(isA, e, 0.0), axis=-1, keepdims=True)
            lB = jnp.sum(jnp.where(isA, 0.0, e), axis=-1, keepdims=True)
            e48 = jnp.concatenate([e, jnp.zeros((8, NK), f32)], axis=0).astype(bf16)
            return e48, 1.0 / lA, 1.0 / lB

        def pv(p, pr, vt, vm):
            e48, rA, rB = pr
            vbd = blockdiag(vt, vm)
            o = jnp.dot(e48, vbd, preferred_element_type=f32)[:SEG + M]
            o = jnp.concatenate([o[:, 0:128] * rA, o[:, 128:256] * jnp.where(lo40, rA, rB),
                                 o[:, 256:384] * rB], axis=1)
            if carry_o is None:
                handed[p] = o[RIDE:SEG]
                return jnp.concatenate([o[:RIDE], o[SEG:SEG + M]], axis=0).astype(bf16)
            return jnp.concatenate([carry_o[p], o], axis=0).astype(bf16)

        def wo(p, lhs2):
            return jnp.dot(lhs2, _as_bf16(wo32[p * DH:(p + 1) * DH, :]), preferred_element_type=f32)

        st = {}
        acc = None
        pend = {}

        def preload(op, p):
            if op == 's':
                pend[(op, p)] = (tok(0, p), tok(1, p))
            elif op == 'pv':
                pend[(op, p)] = tok(2, p)

        producer = {'s': 'qk', 'pv': 'v'}
        done = set()
        for n, (op, p) in enumerate(order):
            for fn in extra.get(n, ()):
                fn()
            if op in ('qk', 'v'):
                for op2, p2 in order[n + 1:n + 6]:
                    if op2 in producer and (op2, p2) not in pend and (producer[op2], p2) in done:
                        preload(op2, p2)
            if op in producer and (op, p) not in pend:
                preload(op, p)
            if op == 'qk':
                st[('q', p)] = proj(0, p)
                st[('k', p)] = proj(1, p)
            elif op == 'v':
                st[('v', p)] = proj(2, p)
            elif op == 's':
                qt, kt = pend.pop((op, p))
                st[('pr', p)] = scores(qt, kt, st.pop(('q', p)), st.pop(('k', p)))
            elif op == 'pv':
                st[('l2', p)] = pv(p, st.pop(('pr', p)), pend.pop((op, p)), st.pop(('v', p)))
            elif op == 'wo':
                w = wo(p, st.pop(('l2', p)))
                acc = w if acc is None else acc + w
            done.add((op, p))

        nt = acc.shape[0] - M
        return acc[:nt], acc[nt:].astype(bf16).astype(f32), handed

    class FFN:
        def __init__(self, r, h):
            self.r = r
            h = h.astype(bf16).astype(f32)
            self.hn = _ln(h).astype(bf16)
            self.acc = h
            self.a = {}

        def gu(self, k):
            g = jnp.dot(self.hn, wg_v[:, k * FC:(k + 1) * FC], preferred_element_type=f32)
            u = jnp.dot(self.hn, wu_v[:, k * FC:(k + 1) * FC], preferred_element_type=f32)
            self.a[k] = (g * jax.nn.sigmoid(g) * u).astype(bf16)

        def down(self, k):
            self.acc = self.acc + jnp.dot(self.a.pop(k), wd_v[k * FC:(k + 1) * FC, :],
                                          preferred_element_type=f32)

        def finish(self):
            out_v[pl.ds(self.r, FB), :] = self.acc.astype(bf16)

    P = functools.partial
    MID = len(order) // 2

    def double_step(d, mem, extra0, extra1):
        a0, mem, handed = segment(2 * d, mem, None, extra0)
        a1, mem, _ = segment(2 * d + 1, mem, handed, extra1)
        r = pl.multiple_of(d * FB, FB)
        h = x_v[pl.ds(r, FB), :].astype(f32) + jnp.concatenate([a0, a1], axis=0)
        return h, mem

    def super_step(j, carry):
        @pl.when(j == 1)
        def _():
            out_copy(0, FB).start()

        @pl.when(j >= 2)
        def _():
            out_copy(pl.multiple_of((2 * j - 3) * FB, FB), 2 * FB).start()
        mem = mem_v[...]
        fa = FFN(pl.multiple_of(jnp.maximum(2 * j - 1, 0) * FB, FB), h_v[...])
        h, mem = double_step(2 * j, mem,
                             {8: [P(fa.gu, 0)]},
                             {0: [P(fa.gu, 1)], MID: [P(fa.down, 0)]})
        fb = FFN(pl.multiple_of(2 * j * FB, FB), h)
        h, mem = double_step(2 * j + 1, mem,
                             {0: [P(fa.down, 1), fa.finish], 12: [P(fb.gu, 0)]},
                             {0: [P(fb.gu, 1)], 16: [P(fb.down, 0)], MID + 8: [P(fb.down, 1), fb.finish]})
        h_v[...] = h
        mem_v[...] = mem
        return carry

    NSUP = NSEG // 4
    lax.fori_loop(0, NSUP, super_step, 0)

    out_copy(S - 3 * FB, 2 * FB).start()
    ffn = FFN(S - FB, h_v[...])
    ffn.gu(0)
    ffn.gu(1)
    ffn.down(0)
    ffn.down(1)
    ffn.finish()
    out_copy(S - FB, FB).start()
    out_copy(0, S).wait()


@jax.jit
def pallas_sequential_preLN__memory_aug_recurrent_mem_tr__swiglu_ffn__prompt_kernel(A_x, A_mem0, A_Wq, A_Wk, A_Wv, A_Wo, A_seg_len, B_x, B_w_gate, B_w_up, B_w_down):
    del A_seg_len, B_x
    x = A_x.reshape(S, D)
    mem0 = A_mem0.reshape(M, D)
    wqt = jnp.transpose(A_Wq, (1, 2, 0)).reshape(HD, D)
    wkt = jnp.transpose(A_Wk, (1, 2, 0)).reshape(HD, D)
    wvt = jnp.transpose(A_Wv, (1, 2, 0)).reshape(HD, D)
    wo = A_Wo.reshape(HD, D)
    any_spec = pl.BlockSpec(memory_space=pl.ANY)
    out = pl.pallas_call(
        _kernel,
        out_shape=jax.ShapeDtypeStruct((S, D), bf16),
        in_specs=[any_spec, pl.BlockSpec(memory_space=pltpu.VMEM)] + [any_spec] * 7,
        out_specs=any_spec,
        scratch_shapes=[
            pltpu.VMEM((S, D), bf16),
            pltpu.VMEM((S, D), bf16),
            pltpu.VMEM((NBUF, CH, D), bf16),
            pltpu.VMEM((D // 2, 3 * HD), u32),
            pltpu.VMEM((HD, D), bf16),
            pltpu.VMEM((HD // 2, D), u32),
            pltpu.VMEM((D, F), bf16),
            pltpu.VMEM((D, F), bf16),
            pltpu.VMEM((F, D), bf16),
            pltpu.VMEM((RING, 3 * HD), bf16),
            pltpu.VMEM((FB, D), f32),
            pltpu.VMEM((M, D), f32),
            pltpu.VMEM((S, D), bf16),
            pltpu.SemaphoreType.DMA((4,)),
            pltpu.SemaphoreType.DMA((NBUF,)),
            pltpu.SemaphoreType.DMA((NCH,)),
            pltpu.SemaphoreType.DMA((3,)),
            pltpu.SemaphoreType.DMA((1,)),
        ],
        compiler_params=pltpu.CompilerParams(vmem_limit_bytes=110 * 1024 * 1024),
    )(x, mem0, wqt, wkt, wvt, wo, B_w_gate, B_w_up, B_w_down)
    return out.reshape(1, S, D)
```

```python
import functools

import jax
import jax.numpy as jnp
from jax import lax
import jax.experimental.pallas as pl
import jax.experimental.pallas.tpu as pltpu

S = 2048
D = 640
H = 32
DH = 192
HD = H * DH
M = 8
SEG = 32
NSEG = S // SEG
F = 1536
EPS = 1e-5
RIDE = 24
PRO = S - RIDE * NSEG
RING = 576
CH = 2048
CPM = HD // CH
NCHK = 3 * CPM
NBUF = 3
NP = H // 2
PW = 2 * DH
SUB = 4
FB = 2 * SEG
NFS = 2
FC = F // NFS

bf16 = jnp.bfloat16
f32 = jnp.float32
u32 = jnp.uint32


def _ln(x):
    m = jnp.mean(x, axis=-1, keepdims=True)
    xc = x - m
    v = jnp.mean(xc * xc, axis=-1, keepdims=True)
    return xc * lax.rsqrt(v + EPS)


def _as_bf16(w32):
    return pltpu.bitcast(w32, bf16)


def _step_order():
    lag = {'qk': 0, 'v': 1, 's': 1, 'pv': 3, 'wo': 7}
    order = []
    for i in range(NP):
        for op in ('qk', 'pv', 'wo', 's', 'v'):
            if i >= lag[op]:
                order.append((op, i - lag[op]))
    rem = {op: list(range(NP - lag[op], NP)) for op in lag}
    for op in ('v', 'pv', 'wo', 's', 'wo', 'pv', 'wo', 'wo', 'wo', 'pv', 'wo', 'wo'):
        order.append((op, rem[op].pop(0)))
    assert not any(rem.values())
    return order


def _kernel(x_hbm, mem0_hbm, wq_hbm, wk_hbm, wv_hbm, wo_hbm, wg_hbm, wu_hbm, wd_hbm,
            out_hbm,
            x_v, xn_v, stage, wqkv, wo32, wg32, wu32, wd32,
            ring, h_v, mem_v, mem0_v, out_v,
            sem_x, sem_stage, sem_first, sem_wo, sem_ffn, sem_out):
    w_hbms = (wq_hbm, wk_hbm, wv_hbm)
    HC = CH // 2
    X0 = PRO + SUB * RIDE

    def x_copy(i):
        if i == 0:
            return pltpu.make_async_copy(x_hbm.at[pl.ds(0, X0)], x_v.at[pl.ds(0, X0)], sem_x.at[0])
        return pltpu.make_async_copy(x_hbm.at[pl.ds(X0, S - X0)], x_v.at[pl.ds(X0, S - X0)], sem_x.at[1])

    def first_copy(i):
        r = pl.multiple_of(i * HC, HC)
        return pltpu.make_async_copy(wq_hbm.at[pl.ds(r, HC)], stage.at[0, pl.ds(r, HC)], sem_first.at[i])

    def w_copy(mat, c, slot):
        return pltpu.make_async_copy(
            w_hbms[mat].at[pl.ds(pl.multiple_of(c * CH, CH), CH)], stage.at[slot], sem_stage.at[slot])

    def wo_copy(c):
        return pltpu.make_async_copy(wo_hbm.at[pl.ds(c * CH, CH)],
                                     wo32.bitcast(bf16).at[pl.ds(c * CH, CH)], sem_wo.at[c])

    def ffn_copy(i):
        src, dst = ((wg_hbm, wg32), (wu_hbm, wu32), (wd_hbm, wd32))[i]
        return pltpu.make_async_copy(src, dst.bitcast(bf16), sem_ffn.at[i])

    def out_copy(r, n):
        return pltpu.make_async_copy(out_v.at[pl.ds(r, n)], out_hbm.at[pl.ds(r, n)], sem_out.at[0])

    def ln_rows(r, n):
        xn_v[pl.ds(r, n), :] = _ln(x_v[pl.ds(r, n), :].astype(f32)).astype(bf16)

    def project_prologue(blk, col, n):
        y = lax.dot_general(xn_v[pl.ds(0, PRO), :], blk, (((1,), (1,)), ((), ())), preferred_element_type=f32)
        ring[pl.ds(RING - PRO, PRO), pl.ds(col, n)] = y.astype(bf16)
        wqkv[:, pl.ds(col, n)] = pltpu.bitcast(blk.T, u32)

    x_copy(0).start()
    first_copy(0).start()
    mem0_copy = pltpu.make_async_copy(mem0_hbm, mem0_v, sem_x.at[2])
    mem0_copy.start()
    h_v[...] = jnp.zeros((FB, D), f32)
    x_copy(0).wait()
    ln_rows(0, X0)

    def pro_a(i, carry):
        first_copy(i).wait()

        @pl.when(i == 0)
        def _():
            first_copy(1).start()
        w_copy(0, i + 1, i + 1).start()
        r = pl.multiple_of(i * HC, HC)
        project_prologue(stage[0, pl.ds(r, HC), :], r, HC)
        return carry

    lax.fori_loop(0, 2, pro_a, 0)

    def pro_b(g, carry):
        slot = g % NBUF
        nslot = (g + 2) % NBUF
        w_copy(0, 0, slot).wait()
        for mat in (1, 2):
            @pl.when((g + 2) // CPM == mat)
            def _(mat=mat):
                w_copy(mat, g + 2 - mat * CPM, nslot).start()
        side = [x_copy(1), wo_copy(0), wo_copy(1), wo_copy(2), ffn_copy(0), ffn_copy(1), ffn_copy(2)]
        for k, cp in enumerate(side):
            @pl.when(g == k + 1)
            def _(cp=cp):
                cp.start()
        project_prologue(stage[slot], pl.multiple_of(g * CH, CH), CH)
        return carry

    lax.fori_loop(1, NCHK, pro_b, 0)

    x_copy(1).wait()
    mem0_copy.wait()
    mem_v[...] = mem0_v[...].astype(f32)
    for i in range(3):
        wo_copy(i).wait()
        ffn_copy(i).wait()

    scale = DH ** (-0.5)
    L = SEG + M
    NK = 2 * L
    lane = lax.broadcasted_iota(jnp.int32, (L, NK), 1)
    row = lax.broadcasted_iota(jnp.int32, (L, NK), 0)
    isA = lane < L
    tokidx = jnp.where(isA, lane, lane - (SEG + 2 * M))
    is_mem_key = (lane >= SEG) & (lane < SEG + 2 * M)
    visible = (row >= SEG) | is_mem_key | (tokidx <= row)
    lo16 = lax.broadcasted_iota(jnp.int32, (SEG // 2, 128), 1) < 64
    lo8 = lax.broadcasted_iota(jnp.int32, (M, 128), 1) < 64
    lo40 = lax.broadcasted_iota(jnp.int32, (L, 128), 1) < 64
    z16 = jnp.zeros((SEG // 2, 128), u32)
    z8 = jnp.zeros((M, 128), f32)
    order = _step_order()

    def blockdiag(t, m):
        t32 = pltpu.bitcast(t, u32)
        t0, t1, t2 = t32[:, 0:128], t32[:, 128:256], t32[:, 256:384]
        top = jnp.concatenate([t0, jnp.where(lo16, t1, jnp.uint32(0)), z16], axis=1)
        bot = jnp.concatenate([z16, jnp.where(lo16, jnp.uint32(0), t1), t2], axis=1)
        m0, m1, m2 = m[:, 0:128], m[:, 128:256], m[:, 256:384]
        ma = jnp.concatenate([m0, jnp.where(lo8, m1, 0.0), z8], axis=1)
        mb = jnp.concatenate([z8, jnp.where(lo8, 0.0, m1), m2], axis=1)
        mid = pltpu.bitcast(jnp.concatenate([ma, mb], axis=0).astype(bf16), u32)
        return pltpu.bitcast(jnp.concatenate([top, mid, bot], axis=0), bf16)

    def mm(a, b):
        return lax.dot_general(a, b, (((1,), (0,)), ((), ())), preferred_element_type=f32)

    def segment(s, xn, mem, extra):
        lhs = jnp.concatenate([xn.astype(f32), mem], axis=0).astype(bf16)
        wslot = pl.multiple_of((RIDE * s) % RING, 8)
        rslot = pl.multiple_of((SEG * s + RING - PRO) % RING, 32)

        def proj(mat, p):
            col = mat * HD + p * PW
            y = mm(lhs, _as_bf16(wqkv[:, col:col + PW]))
            ring[pl.ds(wslot, RIDE), col:col + PW] = y[:RIDE].astype(bf16)
            return y[RIDE:]

        def tok(mat, p):
            col = mat * HD + p * PW
            return ring[pl.ds(rslot, SEG), col:col + PW]

        def scores(qt, kt, qm, km):
            q40 = jnp.concatenate([qt.astype(f32), qm], axis=0)
            kbd = blockdiag(kt, km)
            sc = lax.dot_general(q40, kbd, (((1,), (1,)), ((), ())), preferred_element_type=f32)
            sc = sc * scale
            sc = jnp.where(visible, sc, -1e9)
            mA = jnp.max(jnp.where(isA, sc, -jnp.inf), axis=-1, keepdims=True)
            mB = jnp.max(jnp.where(isA, -jnp.inf, sc), axis=-1, keepdims=True)
            e = jnp.exp(sc - jnp.where(isA, mA, mB))
            lA = jnp.sum(jnp.where(isA, e, 0.0), axis=-1, keepdims=True)
            lB = jnp.sum(jnp.where(isA, 0.0, e), axis=-1, keepdims=True)
            return e, 1.0 / lA, 1.0 / lB

        def pv(pr, vt, vm):
            e, rA, rB = pr
            o = mm(e, blockdiag(vt, vm))
            return jnp.concatenate([o[:, 0:128] * rA, o[:, 128:256] * jnp.where(lo40, rA, rB),
                                    o[:, 256:384] * rB], axis=1)

        def wo(p, o):
            return mm(o, _as_bf16(wo32[p * DH:(p + 1) * DH, :]))

        st = {}
        pend = {}
        acc = None

        def preload(op, p):
            pend[(op, p)] = (tok(0, p), tok(1, p)) if op == 's' else tok(2, p)

        producer = {'s': 'qk', 'pv': 'v'}
        done = set()
        for n, (op, p) in enumerate(order):
            for fn in extra.get(n, ()):
                fn()
            if op in ('qk', 'v'):
                for op2, p2 in order[n + 1:n + 6]:
                    if op2 in producer and (op2, p2) not in pend and (producer[op2], p2) in done:
                        preload(op2, p2)
            if op in producer and (op, p) not in pend:
                preload(op, p)
            if op == 'qk':
                st[('q', p)] = proj(0, p)
                st[('k', p)] = proj(1, p)
            elif op == 'v':
                st[('v', p)] = proj(2, p)
            elif op == 's':
                qt, kt = pend.pop((op, p))
                st[('pr', p)] = scores(qt, kt, st.pop(('q', p)), st.pop(('k', p)))
            elif op == 'pv':
                st[('o', p)] = pv(st.pop(('pr', p)), pend.pop((op, p)), st.pop(('v', p)))
            else:
                w = wo(p, st.pop(('o', p)))
                acc = w if acc is None else acc + w
            done.add((op, p))

        return acc[:SEG], acc[SEG:].astype(bf16).astype(f32)

    class FFN:
        def __init__(self, r, h):
            self.r = r
            h = h.astype(bf16).astype(f32)
            self.hn = _ln(h).astype(bf16)
            self.acc = h
            self.a = {}

        def gu(self, k):
            g = mm(self.hn, _as_bf16(wg32[:, k * FC:(k + 1) * FC]))
            u = mm(self.hn, _as_bf16(wu32[:, k * FC:(k + 1) * FC]))
            self.a[k] = (g * jax.nn.sigmoid(g) * u).astype(bf16)

        def down(self, k):
            self.acc = self.acc + mm(self.a.pop(k), _as_bf16(wd32[k * (FC // 2):(k + 1) * (FC // 2), :]))

        def finish(self):
            out_v[pl.ds(self.r, FB), :] = self.acc.astype(bf16)

    P = functools.partial
    MID = len(order) // 2
    NSUP = NSEG // SUB

    def super_step(j, carry):
        @pl.when(j == 1)
        def _():
            out_copy(0, FB).start()

        @pl.when(j >= 2)
        def _():
            out_copy(pl.multiple_of((2 * j - 3) * FB, FB), 2 * FB).start()
        mem = mem_v[...]
        xr = pl.multiple_of(PRO + SUB * RIDE * j, 32)
        xns = [xn_v[pl.ds(pl.multiple_of(xr + k * RIDE, 8), RIDE), :] for k in range(SUB)]
        xr_next = pl.multiple_of(PRO + SUB * RIDE * jnp.minimum(j + 1, NSUP - 1), 32)

        def double_step(dd, mem, extra0, extra1):
            d = 2 * j + dd
            a0, mem = segment(2 * d, xns[2 * dd], mem, extra0)
            a1, mem = segment(2 * d + 1, xns[2 * dd + 1], mem, extra1)
            r = pl.multiple_of(d * FB, FB)
            h = x_v[pl.ds(r, FB), :].astype(f32) + jnp.concatenate([a0, a1], axis=0)
            return h, mem

        fa = FFN(pl.multiple_of(jnp.maximum(2 * j - 1, 0) * FB, FB), h_v[...])
        h, mem = double_step(0, mem,
                             {8: [P(fa.gu, 0)], MID: [P(ln_rows, xr_next, SUB * RIDE)]},
                             {0: [P(fa.gu, 1)], MID: [P(fa.down, 0)]})
        fb = FFN(pl.multiple_of(2 * j * FB, FB), h)
        h, mem = double_step(1, mem,
                             {0: [P(fa.down, 1), fa.finish], 12: [P(fb.gu, 0)]},
                             {0: [P(fb.gu, 1)], 16: [P(fb.down, 0)], MID + 8: [P(fb.down, 1), fb.finish]})
        h_v[...] = h
        mem_v[...] = mem
        return carry

    lax.fori_loop(0, NSUP, super_step, 0)

    out_copy(S - 3 * FB, 2 * FB).start()
    ffn = FFN(S - FB, h_v[...])
    ffn.gu(0)
    ffn.gu(1)
    ffn.down(0)
    ffn.down(1)
    ffn.finish()
    out_copy(S - FB, FB).start()
    out_copy(0, S).wait()


@jax.jit
def pallas_sequential_preLN__memory_aug_recurrent_mem_tr__swiglu_ffn__prompt_kernel(
        A_x, A_mem0, A_Wq, A_Wk, A_Wv, A_Wo, A_seg_len, B_x, B_w_gate, B_w_up, B_w_down):
    del A_seg_len, B_x
    x = A_x.reshape(S, D)
    mem0 = A_mem0.reshape(M, D)
    wqt = jnp.transpose(A_Wq, (1, 2, 0)).reshape(HD, D)
    wkt = jnp.transpose(A_Wk, (1, 2, 0)).reshape(HD, D)
    wvt = jnp.transpose(A_Wv, (1, 2, 0)).reshape(HD, D)
    wo = A_Wo.reshape(HD, D)
    any_spec = pl.BlockSpec(memory_space=pl.ANY)
    out = pl.pallas_call(
        _kernel,
        out_shape=jax.ShapeDtypeStruct((S, D), bf16),
        in_specs=[any_spec] * 9,
        out_specs=any_spec,
        scratch_shapes=[
            pltpu.VMEM((S, D), bf16),
            pltpu.VMEM((S, D), bf16),
            pltpu.VMEM((NBUF, CH, D), bf16),
            pltpu.VMEM((D // 2, 3 * HD), u32),
            pltpu.VMEM((HD // 2, D), u32),
            pltpu.VMEM((D // 2, F), u32),
            pltpu.VMEM((D // 2, F), u32),
            pltpu.VMEM((F // 2, D), u32),
            pltpu.VMEM((RING, 3 * HD), bf16),
            pltpu.VMEM((FB, D), f32),
            pltpu.VMEM((M, D), f32),
            pltpu.VMEM((M, D), bf16),
            pltpu.VMEM((S, D), bf16),
            pltpu.SemaphoreType.DMA((3,)),
            pltpu.SemaphoreType.DMA((NBUF,)),
            pltpu.SemaphoreType.DMA((2,)),
            pltpu.SemaphoreType.DMA((CPM,)),
            pltpu.SemaphoreType.DMA((3,)),
            pltpu.SemaphoreType.DMA((1,)),
        ],
        compiler_params=pltpu.CompilerParams(vmem_limit_bytes=110 * 1024 * 1024),
    )(x, mem0, wqt, wkt, wvt, wo, B_w_gate, B_w_up, B_w_down)
    return out.reshape(1, S, D)
```

```python
import functools

import jax
import jax.numpy as jnp
from jax import lax
import jax.experimental.pallas as pl
import jax.experimental.pallas.tpu as pltpu

S = 2048
D = 640
H = 32
DH = 192
HD = H * DH
M = 8
SEG = 32
NSEG = S // SEG
F = 1536
EPS = 1e-5
RIDE = 24
PRO = S - RIDE * NSEG
RING = 576
CH = 2048
CPM = HD // CH
NCHK = 3 * CPM
NBUF = 3
NP = H // 2
PW = 2 * DH
SUB = 4
FB = 2 * SEG
NFS = 2
FC = F // NFS

FIRST = ((0, 512), (512, 512), (1024, 1024))

bf16 = jnp.bfloat16
f32 = jnp.float32
u32 = jnp.uint32


def _ln(x):
    m = jnp.mean(x, axis=-1, keepdims=True)
    xc = x - m
    v = jnp.mean(xc * xc, axis=-1, keepdims=True)
    return xc * lax.rsqrt(v + EPS)


def _as_bf16(w32):
    return pltpu.bitcast(w32, bf16)


def _step_order():
    lag = {'qk': 0, 'v': 1, 's': 1, 'pv': 3, 'wo': 7}
    order = []
    for i in range(NP):
        for op in ('qk', 'pv', 'wo', 's', 'v'):
            if i >= lag[op]:
                order.append((op, i - lag[op]))
    rem = {op: list(range(NP - lag[op], NP)) for op in lag}
    for op in ('v', 'pv', 'wo', 's', 'wo', 'pv', 'wo', 'wo', 'wo', 'pv', 'wo', 'wo'):
        order.append((op, rem[op].pop(0)))
    assert not any(rem.values())
    return order


def _kernel(x_hbm, mem0_hbm, wq_hbm, wk_hbm, wv_hbm, wo_hbm, wg_hbm, wu_hbm, wd_hbm,
            out_hbm,
            x_v, xn_v, stage, wqkv, wo32, wg32, wu32, wd32,
            ring, h_v, mem_v, mem0_v, out_v,
            sem_x, sem_stage, sem_first, sem_wo, sem_ffn, sem_out):
    w_hbms = (wq_hbm, wk_hbm, wv_hbm)

    X0 = PRO + SUB * RIDE
    XPIECES = ((0, PRO), (PRO, SUB * RIDE), (X0, S - X0))

    def x_copy(i):
        r, n = XPIECES[i]
        return pltpu.make_async_copy(x_hbm.at[pl.ds(r, n)], x_v.at[pl.ds(r, n)], sem_x.at[i])

    def first_copy(i):
        r, n = FIRST[i]
        return pltpu.make_async_copy(wq_hbm.at[pl.ds(r, n)], stage.at[0, pl.ds(r, n)], sem_first.at[i])

    def w_copy(mat, c, slot):
        return pltpu.make_async_copy(
            w_hbms[mat].at[pl.ds(pl.multiple_of(c * CH, CH), CH)], stage.at[slot], sem_stage.at[slot])

    def wo_copy(c):
        return pltpu.make_async_copy(wo_hbm.at[pl.ds(c * CH, CH)],
                                     wo32.bitcast(bf16).at[pl.ds(c * CH, CH)], sem_wo.at[c])

    def ffn_copy(i):
        src, dst = ((wg_hbm, wg32), (wu_hbm, wu32), (wd_hbm, wd32))[i]
        return pltpu.make_async_copy(src, dst.bitcast(bf16), sem_ffn.at[i])

    def out_copy(r, n):
        return pltpu.make_async_copy(out_v.at[pl.ds(r, n)], out_hbm.at[pl.ds(r, n)], sem_out.at[0])

    def ln_rows(r, n):
        xn_v[pl.ds(r, n), :] = _ln(x_v[pl.ds(r, n), :].astype(f32)).astype(bf16)

    def project_prologue(blk, col, n):
        y = lax.dot_general(xn_v[pl.ds(0, PRO), :], blk, (((1,), (1,)), ((), ())), preferred_element_type=f32)
        ring[pl.ds(RING - PRO, PRO), pl.ds(col, n)] = y.astype(bf16)
        wqkv[:, pl.ds(col, n)] = pltpu.bitcast(blk.T, u32)

    mem0_copy = pltpu.make_async_copy(mem0_hbm, mem0_v, sem_x.at[3])
    mem0_copy.start()
    x_copy(0).start()
    first_copy(0).start()
    h_v[...] = jnp.zeros((FB, D), f32)
    mem0_copy.wait()
    x_copy(1).start()
    mem_v[...] = mem0_v[...].astype(f32)
    x_copy(0).wait()
    for i in range(1, len(FIRST)):
        first_copy(i).start()
    w_copy(0, 1, 1).start()
    w_copy(0, 2, 2).start()
    ln_rows(0, PRO)
    for i, (r, n) in enumerate(FIRST):
        first_copy(i).wait()
        if i == len(FIRST) - 1:
            x_copy(1).wait()
            ln_rows(PRO, SUB * RIDE)
        project_prologue(stage[0, pl.ds(r, n), :], r, n)

    def pro_b(g, carry):
        slot = g % NBUF
        nslot = (g + 2) % NBUF
        w_copy(0, 0, slot).wait()
        for mat in (1, 2):
            @pl.when((g + 2) // CPM == mat)
            def _(mat=mat):
                w_copy(mat, g + 2 - mat * CPM, nslot).start()
        side = [x_copy(2), wo_copy(0), wo_copy(1), wo_copy(2), ffn_copy(0), ffn_copy(1), ffn_copy(2)]
        for k, cp in enumerate(side):
            @pl.when(g == k + 1)
            def _(cp=cp):
                cp.start()
        project_prologue(stage[slot], pl.multiple_of(g * CH, CH), CH)
        return carry

    lax.fori_loop(1, NCHK, pro_b, 0)

    x_copy(2).wait()
    for i in range(3):
        wo_copy(i).wait()
        ffn_copy(i).wait()

    scale = DH ** (-0.5)
    L = SEG + M
    NK = 2 * L
    lane = lax.broadcasted_iota(jnp.int32, (L, NK), 1)
    row = lax.broadcasted_iota(jnp.int32, (L, NK), 0)
    isA = lane < L
    tokidx = jnp.where(isA, lane, lane - (SEG + 2 * M))
    is_mem_key = (lane >= SEG) & (lane < SEG + 2 * M)
    visible = (row >= SEG) | is_mem_key | (tokidx <= row)
    lo16 = lax.broadcasted_iota(jnp.int32, (SEG // 2, 128), 1) < 64
    lo8 = lax.broadcasted_iota(jnp.int32, (M, 128), 1) < 64
    lo40 = lax.broadcasted_iota(jnp.int32, (L, 128), 1) < 64
    z16 = jnp.zeros((SEG // 2, 128), u32)
    z8 = jnp.zeros((M, 128), f32)
    order = _step_order()

    def blockdiag(t, m):
        t32 = pltpu.bitcast(t, u32)
        t0, t1, t2 = t32[:, 0:128], t32[:, 128:256], t32[:, 256:384]
        top = jnp.concatenate([t0, jnp.where(lo16, t1, jnp.uint32(0)), z16], axis=1)
        bot = jnp.concatenate([z16, jnp.where(lo16, jnp.uint32(0), t1), t2], axis=1)
        m0, m1, m2 = m[:, 0:128], m[:, 128:256], m[:, 256:384]
        ma = jnp.concatenate([m0, jnp.where(lo8, m1, 0.0), z8], axis=1)
        mb = jnp.concatenate([z8, jnp.where(lo8, 0.0, m1), m2], axis=1)
        mid = pltpu.bitcast(jnp.concatenate([ma, mb], axis=0).astype(bf16), u32)
        return pltpu.bitcast(jnp.concatenate([top, mid, bot], axis=0), bf16)

    def mm(a, b):
        return lax.dot_general(a, b, (((1,), (0,)), ((), ())), preferred_element_type=f32)

    def segment(s, xn, mem, extra):
        lhs = jnp.concatenate([xn.astype(f32), mem], axis=0).astype(bf16)
        wslot = pl.multiple_of((RIDE * s) % RING, 8)
        rslot = pl.multiple_of((SEG * s + RING - PRO) % RING, 32)

        def proj(mat, p):
            col = mat * HD + p * PW
            y = mm(lhs, _as_bf16(wqkv[:, col:col + PW]))
            ring[pl.ds(wslot, RIDE), col:col + PW] = y[:RIDE].astype(bf16)
            return y[RIDE:]

        def tok(mat, p):
            col = mat * HD + p * PW
            return ring[pl.ds(rslot, SEG), col:col + PW]

        def scores(qt, kt, qm, km):
            q40 = jnp.concatenate([qt.astype(f32), qm], axis=0)
            kbd = blockdiag(kt, km)
            sc = lax.dot_general(q40, kbd, (((1,), (1,)), ((), ())), preferred_element_type=f32)
            sc = sc * scale
            sc = jnp.where(visible, sc, -1e9)
            mA = jnp.max(jnp.where(isA, sc, -jnp.inf), axis=-1, keepdims=True)
            mB = jnp.max(jnp.where(isA, -jnp.inf, sc), axis=-1, keepdims=True)
            e = jnp.exp(sc - jnp.where(isA, mA, mB))
            lA = jnp.sum(jnp.where(isA, e, 0.0), axis=-1, keepdims=True)
            lB = jnp.sum(jnp.where(isA, 0.0, e), axis=-1, keepdims=True)
            return e, 1.0 / lA, 1.0 / lB

        def pv(pr, vt, vm):
            e, rA, rB = pr
            o = mm(e, blockdiag(vt, vm))
            return jnp.concatenate([o[:, 0:128] * rA, o[:, 128:256] * jnp.where(lo40, rA, rB),
                                    o[:, 256:384] * rB], axis=1)

        def wo(p, o):
            return mm(o, _as_bf16(wo32[p * DH:(p + 1) * DH, :]))

        st = {}
        pend = {}
        acc = None

        def preload(op, p):
            pend[(op, p)] = (tok(0, p), tok(1, p)) if op == 's' else tok(2, p)

        producer = {'s': 'qk', 'pv': 'v'}
        done = set()
        for n, (op, p) in enumerate(order):
            for fn in extra.get(n, ()):
                fn()
            if op in ('qk', 'v'):
                for op2, p2 in order[n + 1:n + 6]:
                    if op2 in producer and (op2, p2) not in pend and (producer[op2], p2) in done:
                        preload(op2, p2)
            if op in producer and (op, p) not in pend:
                preload(op, p)
            if op == 'qk':
                st[('q', p)] = proj(0, p)
                st[('k', p)] = proj(1, p)
            elif op == 'v':
                st[('v', p)] = proj(2, p)
            elif op == 's':
                qt, kt = pend.pop((op, p))
                st[('pr', p)] = scores(qt, kt, st.pop(('q', p)), st.pop(('k', p)))
            elif op == 'pv':
                st[('o', p)] = pv(st.pop(('pr', p)), pend.pop((op, p)), st.pop(('v', p)))
            else:
                w = wo(p, st.pop(('o', p)))
                acc = w if acc is None else acc + w
            done.add((op, p))

        return acc[:SEG], acc[SEG:].astype(bf16).astype(f32)

    class FFN:
        def __init__(self, r, h):
            self.r = r
            h = h.astype(bf16).astype(f32)
            self.hn = _ln(h).astype(bf16)
            self.acc = h
            self.a = {}

        def gu(self, k):
            g = mm(self.hn, _as_bf16(wg32[:, k * FC:(k + 1) * FC]))
            u = mm(self.hn, _as_bf16(wu32[:, k * FC:(k + 1) * FC]))
            self.a[k] = (g * jax.nn.sigmoid(g) * u).astype(bf16)

        def down(self, k):
            self.acc = self.acc + mm(self.a.pop(k), _as_bf16(wd32[k * (FC // 2):(k + 1) * (FC // 2), :]))

        def finish(self):
            out_v[pl.ds(self.r, FB), :] = self.acc.astype(bf16)

    P = functools.partial
    MID = len(order) // 2
    NSUP = NSEG // SUB

    def super_step(j, carry):
        @pl.when(j == 1)
        def _():
            out_copy(0, FB).start()

        @pl.when(j >= 2)
        def _():
            out_copy(pl.multiple_of((2 * j - 3) * FB, FB), 2 * FB).start()
        mem = mem_v[...]
        xr = pl.multiple_of(PRO + SUB * RIDE * j, 32)
        xns = [xn_v[pl.ds(pl.multiple_of(xr + k * RIDE, 8), RIDE), :] for k in range(SUB)]
        xr_next = pl.multiple_of(PRO + SUB * RIDE * jnp.minimum(j + 1, NSUP - 1), 32)

        def double_step(dd, mem, extra0, extra1):
            d = 2 * j + dd
            a0, mem = segment(2 * d, xns[2 * dd], mem, extra0)
            a1, mem = segment(2 * d + 1, xns[2 * dd + 1], mem, extra1)
            r = pl.multiple_of(d * FB, FB)
            h = x_v[pl.ds(r, FB), :].astype(f32) + jnp.concatenate([a0, a1], axis=0)
            return h, mem

        fa = FFN(pl.multiple_of(jnp.maximum(2 * j - 1, 0) * FB, FB), h_v[...])
        h, mem = double_step(0, mem,
                             {8: [P(fa.gu, 0)], MID: [P(ln_rows, xr_next, SUB * RIDE)]},
                             {0: [P(fa.gu, 1)], MID: [P(fa.down, 0)]})
        fb = FFN(pl.multiple_of(2 * j * FB, FB), h)
        h, mem = double_step(1, mem,
                             {0: [P(fa.down, 1), fa.finish], 12: [P(fb.gu, 0)]},
                             {0: [P(fb.gu, 1)], 16: [P(fb.down, 0)], MID + 8: [P(fb.down, 1), fb.finish]})
        h_v[...] = h
        mem_v[...] = mem
        return carry

    lax.fori_loop(0, NSUP, super_step, 0)

    out_copy(S - 3 * FB, 2 * FB).start()
    ffn = FFN(S - FB, h_v[...])
    ffn.gu(0)
    ffn.gu(1)
    ffn.down(0)
    ffn.down(1)
    ffn.finish()
    out_copy(S - FB, FB).start()
    out_copy(0, S).wait()


@jax.jit
def pallas_sequential_preLN__memory_aug_recurrent_mem_tr__swiglu_ffn__prompt_kernel(
        A_x, A_mem0, A_Wq, A_Wk, A_Wv, A_Wo, A_seg_len, B_x, B_w_gate, B_w_up, B_w_down):
    del A_seg_len, B_x
    x = A_x.reshape(S, D)
    mem0 = A_mem0.reshape(M, D)
    wqt = jnp.transpose(A_Wq, (1, 2, 0)).reshape(HD, D)
    wkt = jnp.transpose(A_Wk, (1, 2, 0)).reshape(HD, D)
    wvt = jnp.transpose(A_Wv, (1, 2, 0)).reshape(HD, D)
    wo = A_Wo.reshape(HD, D)
    any_spec = pl.BlockSpec(memory_space=pl.ANY)
    out = pl.pallas_call(
        _kernel,
        out_shape=jax.ShapeDtypeStruct((S, D), bf16),
        in_specs=[any_spec] * 9,
        out_specs=any_spec,
        scratch_shapes=[
            pltpu.VMEM((S, D), bf16),
            pltpu.VMEM((S, D), bf16),
            pltpu.VMEM((NBUF, CH, D), bf16),
            pltpu.VMEM((D // 2, 3 * HD), u32),
            pltpu.VMEM((HD // 2, D), u32),
            pltpu.VMEM((D // 2, F), u32),
            pltpu.VMEM((D // 2, F), u32),
            pltpu.VMEM((F // 2, D), u32),
            pltpu.VMEM((RING, 3 * HD), bf16),
            pltpu.VMEM((FB, D), f32),
            pltpu.VMEM((M, D), f32),
            pltpu.VMEM((M, D), bf16),
            pltpu.VMEM((S, D), bf16),
            pltpu.SemaphoreType.DMA((4,)),
            pltpu.SemaphoreType.DMA((NBUF,)),
            pltpu.SemaphoreType.DMA((len(FIRST),)),
            pltpu.SemaphoreType.DMA((CPM,)),
            pltpu.SemaphoreType.DMA((3,)),
            pltpu.SemaphoreType.DMA((1,)),
        ],
        compiler_params=pltpu.CompilerParams(vmem_limit_bytes=110 * 1024 * 1024),
    )(x, mem0, wqt, wkt, wvt, wo, B_w_gate, B_w_up, B_w_down)
    return out.reshape(1, S, D)
```

```python
import functools

import jax
import jax.numpy as jnp
from jax import lax
import jax.experimental.pallas as pl
import jax.experimental.pallas.tpu as pltpu

S = 2048
D = 640
H = 32
DH = 192
HD = H * DH
M = 8
SEG = 32
NSEG = S // SEG
F = 1536
EPS = 1e-5
RIDE = 24
PRO = S - RIDE * NSEG
RING = 576
CH = 2048
CPM = HD // CH
NCHK = 3 * CPM
NBUF = 3
NP = H // 2
PW = 2 * DH
SUB = 4
FB = 2 * SEG
NFS = 2
FC = F // NFS

NFIRST = 4
FP = CH // NFIRST

bf16 = jnp.bfloat16
f32 = jnp.float32
u32 = jnp.uint32


def _ln(x):
    m = jnp.mean(x, axis=-1, keepdims=True)
    xc = x - m
    v = jnp.mean(xc * xc, axis=-1, keepdims=True)
    return xc * lax.rsqrt(v + EPS)


def _as_bf16(w32):
    return pltpu.bitcast(w32, bf16)


def _step_order():
    lag = {'qk': 0, 'v': 1, 's': 1, 'pv': 3, 'wo': 7}
    order = []
    for i in range(NP):
        for op in ('qk', 'pv', 'wo', 's', 'v'):
            if i >= lag[op]:
                order.append((op, i - lag[op]))
    rem = {op: list(range(NP - lag[op], NP)) for op in lag}
    for op in ('v', 'pv', 'wo', 's', 'wo', 'pv', 'wo', 'wo', 'wo', 'pv', 'wo', 'wo'):
        order.append((op, rem[op].pop(0)))
    assert not any(rem.values())
    return order


def _kernel(x_hbm, mem0_hbm, wq_hbm, wk_hbm, wv_hbm, wo_hbm, wg_hbm, wu_hbm, wd_hbm,
            out_hbm,
            x_v, xn_v, stage, wqkv, wo32, wg32, wu32, wd32,
            ring, h_v, mem_v, mem0_v, out_v,
            sem_x, sem_stage, sem_first, sem_wo, sem_ffn, sem_out):
    w_hbms = (wq_hbm, wk_hbm, wv_hbm)

    X0 = PRO + SUB * RIDE
    XPIECES = ((0, X0), (X0, S - X0))

    def x_copy(i):
        r, n = XPIECES[i]
        return pltpu.make_async_copy(x_hbm.at[pl.ds(r, n)], x_v.at[pl.ds(r, n)], sem_x.at[i])

    def first_copy(i):
        r = pl.multiple_of(i * FP, FP)
        return pltpu.make_async_copy(wq_hbm.at[pl.ds(r, FP)], stage.at[0, pl.ds(r, FP)], sem_first.at[i])

    def w_copy(mat, c, slot):
        return pltpu.make_async_copy(
            w_hbms[mat].at[pl.ds(pl.multiple_of(c * CH, CH), CH)], stage.at[slot], sem_stage.at[slot])

    def wo_copy(c):
        return pltpu.make_async_copy(wo_hbm.at[pl.ds(c * CH, CH)],
                                     wo32.bitcast(bf16).at[pl.ds(c * CH, CH)], sem_wo.at[c])

    def ffn_copy(i):
        src, dst = ((wg_hbm, wg32), (wu_hbm, wu32), (wd_hbm, wd32))[i]
        return pltpu.make_async_copy(src, dst.bitcast(bf16), sem_ffn.at[i])

    def out_copy(r, n):
        return pltpu.make_async_copy(out_v.at[pl.ds(r, n)], out_hbm.at[pl.ds(r, n)], sem_out.at[0])

    def ln_rows(r, n):
        xn_v[pl.ds(r, n), :] = _ln(x_v[pl.ds(r, n), :].astype(f32)).astype(bf16)

    def project_prologue(blk, col, n):
        y = lax.dot_general(xn_v[pl.ds(0, PRO), :], blk, (((1,), (1,)), ((), ())), preferred_element_type=f32)
        ring[pl.ds(RING - PRO, PRO), pl.ds(col, n)] = y.astype(bf16)
        wqkv[:, pl.ds(col, n)] = pltpu.bitcast(blk.T, u32)

    mem0_copy = pltpu.make_async_copy(mem0_hbm, mem0_v, sem_x.at[2])
    mem0_copy.start()
    x_copy(0).start()
    h_v[...] = jnp.zeros((FB, D), f32)
    mem0_copy.wait()
    for i in range(NFIRST):
        first_copy(i).start()
    w_copy(0, 1, 1).start()
    w_copy(0, 2, 2).start()
    mem_v[...] = mem0_v[...].astype(f32)
    x_copy(0).wait()
    ln_rows(0, X0)

    def pro_a(i, carry):
        first_copy(i).wait()
        r = pl.multiple_of(i * FP, FP)
        project_prologue(stage[0, pl.ds(r, FP), :], r, FP)
        return carry

    lax.fori_loop(0, NFIRST, pro_a, 0)

    def pro_b(g, carry):
        slot = g % NBUF
        nslot = (g + 2) % NBUF
        w_copy(0, 0, slot).wait()
        for mat in (1, 2):
            @pl.when((g + 2) // CPM == mat)
            def _(mat=mat):
                w_copy(mat, g + 2 - mat * CPM, nslot).start()
        side = [x_copy(1), wo_copy(0), wo_copy(1), wo_copy(2), ffn_copy(0), ffn_copy(1), ffn_copy(2)]
        for k, cp in enumerate(side):
            @pl.when(g == k + 1)
            def _(cp=cp):
                cp.start()
        project_prologue(stage[slot], pl.multiple_of(g * CH, CH), CH)
        return carry

    lax.fori_loop(1, NCHK, pro_b, 0)

    x_copy(1).wait()
    for i in range(3):
        wo_copy(i).wait()
        ffn_copy(i).wait()

    scale = DH ** (-0.5)
    L = SEG + M
    NK = 2 * L
    lane = lax.broadcasted_iota(jnp.int32, (L, NK), 1)
    row = lax.broadcasted_iota(jnp.int32, (L, NK), 0)
    isA = lane < L
    tokidx = jnp.where(isA, lane, lane - (SEG + 2 * M))
    is_mem_key = (lane >= SEG) & (lane < SEG + 2 * M)
    visible = (row >= SEG) | is_mem_key | (tokidx <= row)
    lo16 = lax.broadcasted_iota(jnp.int32, (SEG // 2, 128), 1) < 64
    lo8 = lax.broadcasted_iota(jnp.int32, (M, 128), 1) < 64
    lo40 = lax.broadcasted_iota(jnp.int32, (L, 128), 1) < 64
    z16 = jnp.zeros((SEG // 2, 128), u32)
    z8 = jnp.zeros((M, 128), f32)
    order = _step_order()

    def blockdiag(t, m):
        t32 = pltpu.bitcast(t, u32)
        t0, t1, t2 = t32[:, 0:128], t32[:, 128:256], t32[:, 256:384]
        top = jnp.concatenate([t0, jnp.where(lo16, t1, jnp.uint32(0)), z16], axis=1)
        bot = jnp.concatenate([z16, jnp.where(lo16, jnp.uint32(0), t1), t2], axis=1)
        m0, m1, m2 = m[:, 0:128], m[:, 128:256], m[:, 256:384]
        ma = jnp.concatenate([m0, jnp.where(lo8, m1, 0.0), z8], axis=1)
        mb = jnp.concatenate([z8, jnp.where(lo8, 0.0, m1), m2], axis=1)
        mid = pltpu.bitcast(jnp.concatenate([ma, mb], axis=0).astype(bf16), u32)
        return pltpu.bitcast(jnp.concatenate([top, mid, bot], axis=0), bf16)

    def mm(a, b):
        return lax.dot_general(a, b, (((1,), (0,)), ((), ())), preferred_element_type=f32)

    def segment(s, xn, mem, extra):
        lhs = jnp.concatenate([xn.astype(f32), mem], axis=0).astype(bf16)
        wslot = pl.multiple_of((RIDE * s) % RING, 8)
        rslot = pl.multiple_of((SEG * s + RING - PRO) % RING, 32)

        def proj(mat, p):
            col = mat * HD + p * PW
            y = mm(lhs, _as_bf16(wqkv[:, col:col + PW]))
            ring[pl.ds(wslot, RIDE), col:col + PW] = y[:RIDE].astype(bf16)
            return y[RIDE:]

        def tok(mat, p):
            col = mat * HD + p * PW
            return ring[pl.ds(rslot, SEG), col:col + PW]

        def scores(qt, kt, qm, km):
            q40 = jnp.concatenate([qt.astype(f32), qm], axis=0)
            kbd = blockdiag(kt, km)
            sc = lax.dot_general(q40, kbd, (((1,), (1,)), ((), ())), preferred_element_type=f32)
            sc = sc * scale
            sc = jnp.where(visible, sc, -1e9)
            mA = jnp.max(jnp.where(isA, sc, -jnp.inf), axis=-1, keepdims=True)
            mB = jnp.max(jnp.where(isA, -jnp.inf, sc), axis=-1, keepdims=True)
            e = jnp.exp(sc - jnp.where(isA, mA, mB))
            lA = jnp.sum(jnp.where(isA, e, 0.0), axis=-1, keepdims=True)
            lB = jnp.sum(jnp.where(isA, 0.0, e), axis=-1, keepdims=True)
            return e, 1.0 / lA, 1.0 / lB

        def pv(pr, vt, vm):
            e, rA, rB = pr
            o = mm(e, blockdiag(vt, vm))
            return jnp.concatenate([o[:, 0:128] * rA, o[:, 128:256] * jnp.where(lo40, rA, rB),
                                    o[:, 256:384] * rB], axis=1)

        def wo(p, o):
            return mm(o, _as_bf16(wo32[p * DH:(p + 1) * DH, :]))

        st = {}
        pend = {}
        acc = None

        def preload(op, p):
            pend[(op, p)] = (tok(0, p), tok(1, p)) if op == 's' else tok(2, p)

        producer = {'s': 'qk', 'pv': 'v'}
        done = set()
        for n, (op, p) in enumerate(order):
            for fn in extra.get(n, ()):
                fn()
            if op in ('qk', 'v'):
                for op2, p2 in order[n + 1:n + 6]:
                    if op2 in producer and (op2, p2) not in pend and (producer[op2], p2) in done:
                        preload(op2, p2)
            if op in producer and (op, p) not in pend:
                preload(op, p)
            if op == 'qk':
                st[('q', p)] = proj(0, p)
                st[('k', p)] = proj(1, p)
            elif op == 'v':
                st[('v', p)] = proj(2, p)
            elif op == 's':
                qt, kt = pend.pop((op, p))
                st[('pr', p)] = scores(qt, kt, st.pop(('q', p)), st.pop(('k', p)))
            elif op == 'pv':
                st[('o', p)] = pv(st.pop(('pr', p)), pend.pop((op, p)), st.pop(('v', p)))
            else:
                w = wo(p, st.pop(('o', p)))
                acc = w if acc is None else acc + w
            done.add((op, p))

        return acc[:SEG], acc[SEG:].astype(bf16).astype(f32)

    class FFN:
        def __init__(self, r, h):
            self.r = r
            h = h.astype(bf16).astype(f32)
            self.hn = _ln(h).astype(bf16)
            self.acc = h
            self.a = {}

        def gu(self, k):
            g = mm(self.hn, _as_bf16(wg32[:, k * FC:(k + 1) * FC]))
            u = mm(self.hn, _as_bf16(wu32[:, k * FC:(k + 1) * FC]))
            self.a[k] = (g * jax.nn.sigmoid(g) * u).astype(bf16)

        def down(self, k):
            self.acc = self.acc + mm(self.a.pop(k), _as_bf16(wd32[k * (FC // 2):(k + 1) * (FC // 2), :]))

        def finish(self):
            out_v[pl.ds(self.r, FB), :] = self.acc.astype(bf16)

    P = functools.partial
    MID = len(order) // 2
    NSUP = NSEG // SUB

    def super_step(j, carry):
        @pl.when(j == 1)
        def _():
            out_copy(0, FB).start()

        @pl.when(j >= 2)
        def _():
            out_copy(pl.multiple_of((2 * j - 3) * FB, FB), 2 * FB).start()
        mem = mem_v[...]
        xr = pl.multiple_of(PRO + SUB * RIDE * j, 32)
        xns = [xn_v[pl.ds(pl.multiple_of(xr + k * RIDE, 8), RIDE), :] for k in range(SUB)]
        xr_next = pl.multiple_of(PRO + SUB * RIDE * jnp.minimum(j + 1, NSUP - 1), 32)

        def double_step(dd, mem, extra0, extra1):
            d = 2 * j + dd
            a0, mem = segment(2 * d, xns[2 * dd], mem, extra0)
            a1, mem = segment(2 * d + 1, xns[2 * dd + 1], mem, extra1)
            r = pl.multiple_of(d * FB, FB)
            h = x_v[pl.ds(r, FB), :].astype(f32) + jnp.concatenate([a0, a1], axis=0)
            return h, mem

        fa = FFN(pl.multiple_of(jnp.maximum(2 * j - 1, 0) * FB, FB), h_v[...])
        h, mem = double_step(0, mem,
                             {8: [P(fa.gu, 0)], MID: [P(ln_rows, xr_next, SUB * RIDE)]},
                             {0: [P(fa.gu, 1)], MID: [P(fa.down, 0)]})
        fb = FFN(pl.multiple_of(2 * j * FB, FB), h)
        h, mem = double_step(1, mem,
                             {0: [P(fa.down, 1), fa.finish], 12: [P(fb.gu, 0)]},
                             {0: [P(fb.gu, 1)], 16: [P(fb.down, 0)], MID + 8: [P(fb.down, 1), fb.finish]})
        h_v[...] = h
        mem_v[...] = mem
        return carry

    lax.fori_loop(0, NSUP, super_step, 0)

    out_copy(S - 3 * FB, 2 * FB).start()
    ffn = FFN(S - FB, h_v[...])
    ffn.gu(0)
    ffn.gu(1)
    ffn.down(0)
    ffn.down(1)
    ffn.finish()
    out_copy(S - FB, FB).start()
    out_copy(0, S).wait()


@jax.jit
def pallas_sequential_preLN__memory_aug_recurrent_mem_tr__swiglu_ffn__prompt_kernel(
        A_x, A_mem0, A_Wq, A_Wk, A_Wv, A_Wo, A_seg_len, B_x, B_w_gate, B_w_up, B_w_down):
    del A_seg_len, B_x
    x = A_x.reshape(S, D)
    mem0 = A_mem0.reshape(M, D)
    wqt = jnp.transpose(A_Wq, (1, 2, 0)).reshape(HD, D)
    wkt = jnp.transpose(A_Wk, (1, 2, 0)).reshape(HD, D)
    wvt = jnp.transpose(A_Wv, (1, 2, 0)).reshape(HD, D)
    wo = A_Wo.reshape(HD, D)
    any_spec = pl.BlockSpec(memory_space=pl.ANY)
    out = pl.pallas_call(
        _kernel,
        out_shape=jax.ShapeDtypeStruct((S, D), bf16),
        in_specs=[any_spec] * 9,
        out_specs=any_spec,
        scratch_shapes=[
            pltpu.VMEM((S, D), bf16),
            pltpu.VMEM((S, D), bf16),
            pltpu.VMEM((NBUF, CH, D), bf16),
            pltpu.VMEM((D // 2, 3 * HD), u32),
            pltpu.VMEM((HD // 2, D), u32),
            pltpu.VMEM((D // 2, F), u32),
            pltpu.VMEM((D // 2, F), u32),
            pltpu.VMEM((F // 2, D), u32),
            pltpu.VMEM((RING, 3 * HD), bf16),
            pltpu.VMEM((FB, D), f32),
            pltpu.VMEM((M, D), f32),
            pltpu.VMEM((M, D), bf16),
            pltpu.VMEM((S, D), bf16),
            pltpu.SemaphoreType.DMA((3,)),
            pltpu.SemaphoreType.DMA((NBUF,)),
            pltpu.SemaphoreType.DMA((NFIRST,)),
            pltpu.SemaphoreType.DMA((CPM,)),
            pltpu.SemaphoreType.DMA((3,)),
            pltpu.SemaphoreType.DMA((1,)),
        ],
        compiler_params=pltpu.CompilerParams(vmem_limit_bytes=110 * 1024 * 1024),
    )(x, mem0, wqt, wkt, wvt, wo, B_w_gate, B_w_up, B_w_down)
    return out.reshape(1, S, D)
```

```python
import functools

import jax
import jax.numpy as jnp
from jax import lax
import jax.experimental.pallas as pl
import jax.experimental.pallas.tpu as pltpu

S = 2048
D = 640
H = 32
DH = 192
HD = H * DH
M = 8
SEG = 32
NSEG = S // SEG
F = 1536
EPS = 1e-5
RIDE = 24
PRO = S - RIDE * NSEG
RING = 576
CH = 2048
CPM = HD // CH
NCHK = 3 * CPM
NBUF = 3
NP = H // 2
PW = 2 * DH
SUB = 4
NSUP = NSEG // SUB
FB = 2 * SEG
NFS = 2
FC = F // NFS

NFIRST = 4
FP = CH // NFIRST
NWP = 6
WP = HD // NWP
WLAG = NCHK - NWP

bf16 = jnp.bfloat16
f32 = jnp.float32
u32 = jnp.uint32


def _ln(x):
    m = jnp.mean(x, axis=-1, keepdims=True)
    xc = x - m
    v = jnp.mean(xc * xc, axis=-1, keepdims=True)
    return xc * lax.rsqrt(v + EPS)


def _as_bf16(w32):
    return pltpu.bitcast(w32, bf16)


def _step_order():
    lag = {'qk': 0, 'v': 1, 's': 1, 'pv': 3, 'wo': 7}
    order = []
    for i in range(NP):
        for op in ('qk', 'pv', 'wo', 's', 'v'):
            if i >= lag[op]:
                order.append((op, i - lag[op]))
    rem = {op: list(range(NP - lag[op], NP)) for op in lag}
    for op in ('v', 'pv', 'wo', 's', 'wo', 'pv', 'wo', 'wo', 'wo', 'pv', 'wo', 'wo'):
        order.append((op, rem[op].pop(0)))
    assert not any(rem.values())
    return order


def _kernel(x_hbm, mem0_hbm, wq_hbm, wk_hbm, wv_hbm, wo_hbm, wg_hbm, wu_hbm, wd_hbm,
            out_hbm,
            x_v, xn_v, stage, wqkv, wo32, wg_v, wu_v, wd_v,
            ring, h_v, mem_v, mem0_v, out_v,
            sem_x, sem_stage, sem_first, sem_wo, sem_ffn, sem_out):
    w_hbms = (wq_hbm, wk_hbm, wv_hbm)

    X0 = PRO + SUB * RIDE
    XPIECES = ((0, X0), (X0, S - X0))

    def x_copy(i):
        r, n = XPIECES[i]
        return pltpu.make_async_copy(x_hbm.at[pl.ds(r, n)], x_v.at[pl.ds(r, n)], sem_x.at[i])

    def first_copy(i):
        r = pl.multiple_of(i * FP, FP)
        return pltpu.make_async_copy(wq_hbm.at[pl.ds(r, FP)], stage.at[pl.ds(r, FP)], sem_first.at[i])

    def w_copy(mat, c, slot):
        return pltpu.make_async_copy(
            w_hbms[mat].at[pl.ds(pl.multiple_of(c * CH, CH), CH)],
            stage.at[pl.ds(pl.multiple_of(slot * CH, CH), CH)], sem_stage.at[slot])

    def wo_copy(c):
        r = pl.multiple_of(c * WP, WP)
        return pltpu.make_async_copy(wo_hbm.at[pl.ds(r, WP)],
                                     stage.at[pl.ds(pl.multiple_of(NBUF * CH + r, WP), WP)], sem_wo.at[c])

    def ffn_copy(i):
        src, dst = ((wg_hbm, wg_v), (wu_hbm, wu_v), (wd_hbm, wd_v))[i]
        return pltpu.make_async_copy(src, dst, sem_ffn.at[i])

    def out_copy(j):
        if isinstance(j, int) and j == 1:
            r, n = 0, FB
        elif isinstance(j, int) and j == NSUP + 1:
            r, n = S - FB, FB
        else:
            r, n = pl.multiple_of((2 * j - 3) * FB, FB), 2 * FB
        return pltpu.make_async_copy(out_v.at[pl.ds(r, n)], out_hbm.at[pl.ds(r, n)], sem_out.at[j])

    def ln_rows(r, n):
        xn_v[pl.ds(r, n), :] = _ln(x_v[pl.ds(r, n), :].astype(f32)).astype(bf16)

    def project_prologue(blk, col, n):
        y = lax.dot_general(xn_v[pl.ds(0, PRO), :], blk, (((1,), (1,)), ((), ())), preferred_element_type=f32)
        ring[pl.ds(RING - PRO, PRO), pl.ds(col, n)] = y.astype(bf16)
        wqkv[:, pl.ds(col, n)] = pltpu.bitcast(blk.T, u32)

    mem0_copy = pltpu.make_async_copy(mem0_hbm, mem0_v, sem_x.at[2])
    mem0_copy.start()
    x_copy(0).start()
    h_v[...] = jnp.zeros((FB, D), f32)
    mem0_copy.wait()
    for i in range(NFIRST):
        first_copy(i).start()
    w_copy(0, 1, 1).start()
    w_copy(0, 2, 2).start()
    mem_v[...] = mem0_v[...].astype(f32)
    x_copy(0).wait()
    ln_rows(0, X0)

    def pro_a(i, carry):
        first_copy(i).wait()
        r = pl.multiple_of(i * FP, FP)
        project_prologue(stage[pl.ds(r, FP), :], r, FP)
        return carry

    lax.fori_loop(0, NFIRST, pro_a, 0)

    def pro_b(g, carry):
        slot = g % NBUF
        nslot = (g + 2) % NBUF
        w_copy(0, 0, slot).wait()

        @pl.when(g >= WLAG)
        def _():
            wo_copy(g - WLAG).wait()
        for mat in (1, 2):
            @pl.when((g + 2) // CPM == mat)
            def _(mat=mat):
                w_copy(mat, g + 2 - mat * CPM, nslot).start()

        @pl.when(g <= NWP)
        def _():
            wo_copy(g - 1).start()
        side = {1: x_copy(1), 5: ffn_copy(0), 6: ffn_copy(1), 7: ffn_copy(2)}
        for k, cp in side.items():
            @pl.when(g == k)
            def _(cp=cp):
                cp.start()
        srow = pl.multiple_of(slot * CH, CH)
        wsrc = pl.multiple_of(jnp.where(g >= WLAG, NBUF * CH + (g - WLAG) * WP, srow), WP)
        wdst = pl.multiple_of(jnp.maximum(g - WLAG, 0) * (WP // 2), WP // 2)
        wo32[pl.ds(wdst, WP // 2), :] = pltpu.bitcast(stage[pl.ds(wsrc, WP), :], u32)
        project_prologue(stage[pl.ds(srow, CH), :], pl.multiple_of(g * CH, CH), CH)
        return carry

    lax.fori_loop(1, NCHK, pro_b, 0)

    x_copy(1).wait()
    for i in range(3):
        ffn_copy(i).wait()

    scale = DH ** (-0.5)
    L = SEG + M
    NK = 2 * L
    lane = lax.broadcasted_iota(jnp.int32, (L, NK), 1)
    row = lax.broadcasted_iota(jnp.int32, (L, NK), 0)
    isA = lane < L
    tokidx = jnp.where(isA, lane, lane - (SEG + 2 * M))
    is_mem_key = (lane >= SEG) & (lane < SEG + 2 * M)
    visible = (row >= SEG) | is_mem_key | (tokidx <= row)
    lo16 = lax.broadcasted_iota(jnp.int32, (SEG // 2, 128), 1) < 64
    lo8 = lax.broadcasted_iota(jnp.int32, (M, 128), 1) < 64
    lo40 = lax.broadcasted_iota(jnp.int32, (L, 128), 1) < 64
    z16 = jnp.zeros((SEG // 2, 128), u32)
    z8 = jnp.zeros((M, 128), f32)
    order = _step_order()

    def blockdiag(t, m):
        t32 = pltpu.bitcast(t, u32)
        t0, t1, t2 = t32[:, 0:128], t32[:, 128:256], t32[:, 256:384]
        top = jnp.concatenate([t0, jnp.where(lo16, t1, jnp.uint32(0)), z16], axis=1)
        bot = jnp.concatenate([z16, jnp.where(lo16, jnp.uint32(0), t1), t2], axis=1)
        m0, m1, m2 = m[:, 0:128], m[:, 128:256], m[:, 256:384]
        ma = jnp.concatenate([m0, jnp.where(lo8, m1, 0.0), z8], axis=1)
        mb = jnp.concatenate([z8, jnp.where(lo8, 0.0, m1), m2], axis=1)
        mid = pltpu.bitcast(jnp.concatenate([ma, mb], axis=0).astype(bf16), u32)
        return pltpu.bitcast(jnp.concatenate([top, mid, bot], axis=0), bf16)

    def mm(a, b):
        return lax.dot_general(a, b, (((1,), (0,)), ((), ())), preferred_element_type=f32)

    def segment(s, xn, mem, extra):
        lhs = jnp.concatenate([xn.astype(f32), mem], axis=0).astype(bf16)
        wslot = pl.multiple_of((RIDE * s) % RING, 8)
        rslot = pl.multiple_of((SEG * s + RING - PRO) % RING, 32)

        def proj(mat, p):
            col = mat * HD + p * PW
            y = mm(lhs, _as_bf16(wqkv[:, col:col + PW]))
            ring[pl.ds(wslot, RIDE), col:col + PW] = y[:RIDE].astype(bf16)
            return y[RIDE:]

        def tok(mat, p):
            col = mat * HD + p * PW
            return ring[pl.ds(rslot, SEG), col:col + PW]

        def scores(qt, kt, qm, km):
            q40 = jnp.concatenate([qt.astype(f32), qm], axis=0)
            kbd = blockdiag(kt, km)
            sc = lax.dot_general(q40, kbd, (((1,), (1,)), ((), ())), preferred_element_type=f32)
            sc = sc * scale
            sc = jnp.where(visible, sc, -1e9)
            mA = jnp.max(jnp.where(isA, sc, -jnp.inf), axis=-1, keepdims=True)
            mB = jnp.max(jnp.where(isA, -jnp.inf, sc), axis=-1, keepdims=True)
            e = jnp.exp(sc - jnp.where(isA, mA, mB))
            lA = jnp.sum(jnp.where(isA, e, 0.0), axis=-1, keepdims=True)
            lB = jnp.sum(jnp.where(isA, 0.0, e), axis=-1, keepdims=True)
            return e, 1.0 / lA, 1.0 / lB

        def pv(pr, vt, vm):
            e, rA, rB = pr
            o = mm(e, blockdiag(vt, vm))
            return jnp.concatenate([o[:, 0:128] * rA, o[:, 128:256] * jnp.where(lo40, rA, rB),
                                    o[:, 256:384] * rB], axis=1)

        def wo(p, o):
            return mm(o, _as_bf16(wo32[p * DH:(p + 1) * DH, :]))

        st = {}
        pend = {}
        acc = None

        def preload(op, p):
            pend[(op, p)] = (tok(0, p), tok(1, p)) if op == 's' else tok(2, p)

        producer = {'s': 'qk', 'pv': 'v'}
        done = set()
        for n, (op, p) in enumerate(order):
            for fn in extra.get(n, ()):
                fn()
            if op in ('qk', 'v'):
                for op2, p2 in order[n + 1:n + 6]:
                    if op2 in producer and (op2, p2) not in pend and (producer[op2], p2) in done:
                        preload(op2, p2)
            if op in producer and (op, p) not in pend:
                preload(op, p)
            if op == 'qk':
                st[('q', p)] = proj(0, p)
                st[('k', p)] = proj(1, p)
            elif op == 'v':
                st[('v', p)] = proj(2, p)
            elif op == 's':
                qt, kt = pend.pop((op, p))
                st[('pr', p)] = scores(qt, kt, st.pop(('q', p)), st.pop(('k', p)))
            elif op == 'pv':
                st[('o', p)] = pv(st.pop(('pr', p)), pend.pop((op, p)), st.pop(('v', p)))
            else:
                w = wo(p, st.pop(('o', p)))
                acc = w if acc is None else acc + w
            done.add((op, p))

        return acc[:SEG], acc[SEG:].astype(bf16).astype(f32)

    class FFN:
        def __init__(self, r, h):
            self.r = r
            h = h.astype(bf16).astype(f32)
            self.hn = _ln(h).astype(bf16)
            self.acc = h
            self.a = {}

        def gu(self, k):
            g = mm(self.hn, wg_v[:, k * FC:(k + 1) * FC])
            u = mm(self.hn, wu_v[:, k * FC:(k + 1) * FC])
            self.a[k] = (g * jax.nn.sigmoid(g) * u).astype(bf16)

        def down(self, k):
            self.acc = self.acc + mm(self.a.pop(k), wd_v[k * FC:(k + 1) * FC, :])

        def finish(self):
            out_v[pl.ds(self.r, FB), :] = self.acc.astype(bf16)

    P = functools.partial
    MID = len(order) // 2

    def super_step(j, carry):
        @pl.when(j == 1)
        def _():
            out_copy(1).start()

        @pl.when(j >= 2)
        def _():
            out_copy(j).start()
        mem = mem_v[...]
        xr = pl.multiple_of(PRO + SUB * RIDE * j, 32)
        xns = [xn_v[pl.ds(pl.multiple_of(xr + k * RIDE, 8), RIDE), :] for k in range(SUB)]
        xr_next = pl.multiple_of(PRO + SUB * RIDE * jnp.minimum(j + 1, NSUP - 1), 32)

        def double_step(dd, mem, extra0, extra1):
            d = 2 * j + dd
            a0, mem = segment(2 * d, xns[2 * dd], mem, extra0)
            a1, mem = segment(2 * d + 1, xns[2 * dd + 1], mem, extra1)
            r = pl.multiple_of(d * FB, FB)
            h = x_v[pl.ds(r, FB), :].astype(f32) + jnp.concatenate([a0, a1], axis=0)
            return h, mem

        fa = FFN(pl.multiple_of(jnp.maximum(2 * j - 1, 0) * FB, FB), h_v[...])
        h, mem = double_step(0, mem,
                             {8: [P(fa.gu, 0)], MID: [P(ln_rows, xr_next, SUB * RIDE)]},
                             {0: [P(fa.gu, 1)], MID: [P(fa.down, 0)]})
        fb = FFN(pl.multiple_of(2 * j * FB, FB), h)
        h, mem = double_step(1, mem,
                             {0: [P(fa.down, 1), fa.finish], 12: [P(fb.gu, 0)]},
                             {0: [P(fb.gu, 1)], 16: [P(fb.down, 0)], MID + 8: [P(fb.down, 1), fb.finish]})
        h_v[...] = h
        mem_v[...] = mem
        return carry

    lax.fori_loop(0, NSUP, super_step, 0)

    out_copy(NSUP).start()
    ffn = FFN(S - FB, h_v[...])
    ffn.gu(0)
    ffn.gu(1)
    ffn.down(0)
    ffn.down(1)
    ffn.finish()
    out_copy(NSUP + 1).start()
    for j in range(1, NSUP + 2):
        out_copy(j).wait()


@jax.jit
def pallas_sequential_preLN__memory_aug_recurrent_mem_tr__swiglu_ffn__prompt_kernel(
        A_x, A_mem0, A_Wq, A_Wk, A_Wv, A_Wo, A_seg_len, B_x, B_w_gate, B_w_up, B_w_down):
    del A_seg_len, B_x
    x = A_x.reshape(S, D)
    mem0 = A_mem0.reshape(M, D)
    wqt = jnp.transpose(A_Wq, (1, 2, 0)).reshape(HD, D)
    wkt = jnp.transpose(A_Wk, (1, 2, 0)).reshape(HD, D)
    wvt = jnp.transpose(A_Wv, (1, 2, 0)).reshape(HD, D)
    wo = A_Wo.reshape(HD, D)
    any_spec = pl.BlockSpec(memory_space=pl.ANY)
    out = pl.pallas_call(
        _kernel,
        out_shape=jax.ShapeDtypeStruct((S, D), bf16),
        in_specs=[any_spec] * 9,
        out_specs=any_spec,
        scratch_shapes=[
            pltpu.VMEM((S, D), bf16),
            pltpu.VMEM((S, D), bf16),
            pltpu.VMEM((NBUF * CH + HD, D), bf16),
            pltpu.VMEM((D // 2, 3 * HD), u32),
            pltpu.VMEM((HD // 2, D), u32),
            pltpu.VMEM((D, F), bf16),
            pltpu.VMEM((D, F), bf16),
            pltpu.VMEM((F, D), bf16),
            pltpu.VMEM((RING, 3 * HD), bf16),
            pltpu.VMEM((FB, D), f32),
            pltpu.VMEM((M, D), f32),
            pltpu.VMEM((M, D), bf16),
            pltpu.VMEM((S, D), bf16),
            pltpu.SemaphoreType.DMA((3,)),
            pltpu.SemaphoreType.DMA((NBUF,)),
            pltpu.SemaphoreType.DMA((NFIRST,)),
            pltpu.SemaphoreType.DMA((NWP,)),
            pltpu.SemaphoreType.DMA((3,)),
            pltpu.SemaphoreType.DMA((NSUP + 2,)),
        ],
        compiler_params=pltpu.CompilerParams(vmem_limit_bytes=110 * 1024 * 1024, disable_bounds_checks=True, disable_semaphore_checks=True),
    )(x, mem0, wqt, wkt, wvt, wo, B_w_gate, B_w_up, B_w_down)
    return out.reshape(1, S, D)
```

```python
import functools

import jax
import jax.numpy as jnp
from jax import lax
import jax.experimental.pallas as pl
import jax.experimental.pallas.tpu as pltpu

S = 2048
D = 640
H = 32
DH = 192
HD = H * DH
M = 8
SEG = 32
NSEG = S // SEG
F = 1536
EPS = 1e-5
RIDE = 24
PRO = S - RIDE * NSEG
RING = 576
CH = 2048
CPM = HD // CH
NCHK = 3 * CPM
NBUF = 3
NP = H // 2
PW = 2 * DH
SUB = 4
NSUP = NSEG // SUB
NFS = 2
FC = F // NFS

NFIRST = 4
FP = CH // NFIRST
NWP = 6
WP = HD // NWP
WLAG = NCHK - NWP

bf16 = jnp.bfloat16
f32 = jnp.float32
u32 = jnp.uint32


def _ln(x):
    m = jnp.mean(x, axis=-1, keepdims=True)
    xc = x - m
    v = jnp.mean(xc * xc, axis=-1, keepdims=True)
    return xc * lax.rsqrt(v + EPS)


def _as_bf16(w32):
    return pltpu.bitcast(w32, bf16)


def _step_order():
    lag = {'qk': 0, 'v': 1, 's': 1, 'pv': 3, 'wo': 7}
    order = []
    for i in range(NP):
        for op in ('qk', 'pv', 'wo', 's', 'v'):
            if i >= lag[op]:
                order.append((op, i - lag[op]))
    rem = {op: list(range(NP - lag[op], NP)) for op in lag}
    for op in ('v', 'pv', 'wo', 's', 'wo', 'pv', 'wo', 'wo', 'wo', 'pv', 'wo', 'wo'):
        order.append((op, rem[op].pop(0)))
    assert not any(rem.values())
    return order


def _kernel(x_hbm, mem0_hbm, wq_hbm, wk_hbm, wv_hbm, wo_hbm, wg_hbm, wu_hbm, wd_hbm,
            out_hbm,
            x_v, xn_v, stage, wqkv, wo32, wg_v, wu_v, wd_v,
            ring, h_v, mem_v, mem0_v, out_v,
            sem_x, sem_stage, sem_first, sem_wo, sem_ffn, sem_out):
    w_hbms = (wq_hbm, wk_hbm, wv_hbm)

    X0 = PRO + SUB * RIDE
    XPIECES = ((0, X0), (X0, S - X0))

    def x_copy(i):
        r, n = XPIECES[i]
        return pltpu.make_async_copy(x_hbm.at[pl.ds(r, n)], x_v.at[pl.ds(r, n)], sem_x.at[i])

    def first_copy(i):
        r = pl.multiple_of(i * FP, FP)
        return pltpu.make_async_copy(wq_hbm.at[pl.ds(r, FP)], stage.at[pl.ds(r, FP)], sem_first.at[i])

    def w_copy(mat, c, slot):
        return pltpu.make_async_copy(
            w_hbms[mat].at[pl.ds(pl.multiple_of(c * CH, CH), CH)],
            stage.at[pl.ds(pl.multiple_of(slot * CH, CH), CH)], sem_stage.at[slot])

    def wo_copy(c):
        r = pl.multiple_of(c * WP, WP)
        return pltpu.make_async_copy(wo_hbm.at[pl.ds(r, WP)],
                                     stage.at[pl.ds(pl.multiple_of(NBUF * CH + r, WP), WP)], sem_wo.at[c])

    def ffn_copy(i):
        src, dst = ((wg_hbm, wg_v), (wu_hbm, wu_v), (wd_hbm, wd_v))[i]
        return pltpu.make_async_copy(src, dst, sem_ffn.at[i])

    def out_copy(j):
        if isinstance(j, int) and j == 1:
            r, n = 0, 3 * SEG
        elif isinstance(j, int) and j == NSUP + 1:
            r, n = S - SEG, SEG
        else:
            r, n = pl.multiple_of((4 * j - 5) * SEG, SEG), 4 * SEG
        return pltpu.make_async_copy(out_v.at[pl.ds(r, n)], out_hbm.at[pl.ds(r, n)], sem_out.at[j])

    def ln_rows(r, n):
        xn_v[pl.ds(r, n), :] = _ln(x_v[pl.ds(r, n), :].astype(f32)).astype(bf16)

    def project_prologue(blk, col, n):
        y = lax.dot_general(xn_v[pl.ds(0, PRO), :], blk, (((1,), (1,)), ((), ())), preferred_element_type=f32)
        ring[pl.ds(RING - PRO, PRO), pl.ds(col, n)] = y.astype(bf16)
        wqkv[:, pl.ds(col, n)] = pltpu.bitcast(blk.T, u32)

    mem0_copy = pltpu.make_async_copy(mem0_hbm, mem0_v, sem_x.at[2])
    mem0_copy.start()
    x_copy(0).start()
    h_v[...] = jnp.zeros((SEG, D), f32)
    mem0_copy.wait()
    for i in range(NFIRST):
        first_copy(i).start()
    w_copy(0, 1, 1).start()
    w_copy(0, 2, 2).start()
    mem_v[...] = mem0_v[...].astype(f32)
    x_copy(0).wait()
    ln_rows(0, X0)

    def pro_a(i, carry):
        first_copy(i).wait()
        r = pl.multiple_of(i * FP, FP)
        project_prologue(stage[pl.ds(r, FP), :], r, FP)
        return carry

    lax.fori_loop(0, NFIRST, pro_a, 0)

    def pro_b(g, carry):
        slot = g % NBUF
        nslot = (g + 2) % NBUF
        w_copy(0, 0, slot).wait()

        @pl.when(g >= WLAG)
        def _():
            wo_copy(g - WLAG).wait()
        for mat in (1, 2):
            @pl.when((g + 2) // CPM == mat)
            def _(mat=mat):
                w_copy(mat, g + 2 - mat * CPM, nslot).start()

        @pl.when(g <= NWP)
        def _():
            wo_copy(g - 1).start()
        side = {1: x_copy(1), 5: ffn_copy(0), 6: ffn_copy(1), 7: ffn_copy(2)}
        for k, cp in side.items():
            @pl.when(g == k)
            def _(cp=cp):
                cp.start()
        srow = pl.multiple_of(slot * CH, CH)
        wsrc = pl.multiple_of(jnp.where(g >= WLAG, NBUF * CH + (g - WLAG) * WP, srow), WP)
        wdst = pl.multiple_of(jnp.maximum(g - WLAG, 0) * (WP // 2), WP // 2)
        wo32[pl.ds(wdst, WP // 2), :] = pltpu.bitcast(stage[pl.ds(wsrc, WP), :], u32)
        project_prologue(stage[pl.ds(srow, CH), :], pl.multiple_of(g * CH, CH), CH)
        return carry

    lax.fori_loop(1, NCHK, pro_b, 0)

    x_copy(1).wait()
    for i in range(3):
        ffn_copy(i).wait()

    scale = DH ** (-0.5)
    L = SEG + M
    NK = 2 * L
    lane = lax.broadcasted_iota(jnp.int32, (L, NK), 1)
    row = lax.broadcasted_iota(jnp.int32, (L, NK), 0)
    isA = lane < L
    tokidx = jnp.where(isA, lane, lane - (SEG + 2 * M))
    is_mem_key = (lane >= SEG) & (lane < SEG + 2 * M)
    visible = (row >= SEG) | is_mem_key | (tokidx <= row)
    lo16 = lax.broadcasted_iota(jnp.int32, (SEG // 2, 128), 1) < 64
    lo8 = lax.broadcasted_iota(jnp.int32, (M, 128), 1) < 64
    lo40 = lax.broadcasted_iota(jnp.int32, (L, 128), 1) < 64
    z16 = jnp.zeros((SEG // 2, 128), u32)
    z8 = jnp.zeros((M, 128), f32)
    order = _step_order()

    def blockdiag(t, m):
        t32 = pltpu.bitcast(t, u32)
        t0, t1, t2 = t32[:, 0:128], t32[:, 128:256], t32[:, 256:384]
        top = jnp.concatenate([t0, jnp.where(lo16, t1, jnp.uint32(0)), z16], axis=1)
        bot = jnp.concatenate([z16, jnp.where(lo16, jnp.uint32(0), t1), t2], axis=1)
        m0, m1, m2 = m[:, 0:128], m[:, 128:256], m[:, 256:384]
        ma = jnp.concatenate([m0, jnp.where(lo8, m1, 0.0), z8], axis=1)
        mb = jnp.concatenate([z8, jnp.where(lo8, 0.0, m1), m2], axis=1)
        mid = pltpu.bitcast(jnp.concatenate([ma, mb], axis=0).astype(bf16), u32)
        return pltpu.bitcast(jnp.concatenate([top, mid, bot], axis=0), bf16)

    def mm(a, b):
        return lax.dot_general(a, b, (((1,), (0,)), ((), ())), preferred_element_type=f32)

    def segment(s, xn, mem, extra):
        lhs = jnp.concatenate([xn.astype(f32), mem], axis=0).astype(bf16)
        wslot = pl.multiple_of((RIDE * s) % RING, 8)
        rslot = pl.multiple_of((SEG * s + RING - PRO) % RING, 32)

        def proj(mat, p):
            col = mat * HD + p * PW
            y = mm(lhs, _as_bf16(wqkv[:, col:col + PW]))
            ring[pl.ds(wslot, RIDE), col:col + PW] = y[:RIDE].astype(bf16)
            return y[RIDE:]

        def tok(mat, p):
            col = mat * HD + p * PW
            return ring[pl.ds(rslot, SEG), col:col + PW]

        def scores(qt, kt, qm, km):
            q40 = jnp.concatenate([qt.astype(f32), qm], axis=0)
            kbd = blockdiag(kt, km)
            sc = lax.dot_general(q40, kbd, (((1,), (1,)), ((), ())), preferred_element_type=f32)
            sc = sc * scale
            sc = jnp.where(visible, sc, -1e9)
            mA = jnp.max(jnp.where(isA, sc, -jnp.inf), axis=-1, keepdims=True)
            mB = jnp.max(jnp.where(isA, -jnp.inf, sc), axis=-1, keepdims=True)
            e = jnp.exp(sc - jnp.where(isA, mA, mB))
            lA = jnp.sum(jnp.where(isA, e, 0.0), axis=-1, keepdims=True)
            lB = jnp.sum(jnp.where(isA, 0.0, e), axis=-1, keepdims=True)
            return e, 1.0 / lA, 1.0 / lB

        def pv(pr, vt, vm):
            e, rA, rB = pr
            o = mm(e, blockdiag(vt, vm))
            return jnp.concatenate([o[:, 0:128] * rA, o[:, 128:256] * jnp.where(lo40, rA, rB),
                                    o[:, 256:384] * rB], axis=1)

        def wo(p, o):
            return mm(o, _as_bf16(wo32[p * DH:(p + 1) * DH, :]))

        st = {}
        pend = {}
        acc = None

        def preload(op, p):
            pend[(op, p)] = (tok(0, p), tok(1, p)) if op == 's' else tok(2, p)

        producer = {'s': 'qk', 'pv': 'v'}
        done = set()
        for n, (op, p) in enumerate(order):
            for fn in extra.get(n, ()):
                fn()
            if op in ('qk', 'v'):
                for op2, p2 in order[n + 1:n + 6]:
                    if op2 in producer and (op2, p2) not in pend and (producer[op2], p2) in done:
                        preload(op2, p2)
            if op in producer and (op, p) not in pend:
                preload(op, p)
            if op == 'qk':
                st[('q', p)] = proj(0, p)
                st[('k', p)] = proj(1, p)
            elif op == 'v':
                st[('v', p)] = proj(2, p)
            elif op == 's':
                qt, kt = pend.pop((op, p))
                st[('pr', p)] = scores(qt, kt, st.pop(('q', p)), st.pop(('k', p)))
            elif op == 'pv':
                st[('o', p)] = pv(st.pop(('pr', p)), pend.pop((op, p)), st.pop(('v', p)))
            else:
                w = wo(p, st.pop(('o', p)))
                acc = w if acc is None else acc + w
            done.add((op, p))

        return acc[:SEG], acc[SEG:].astype(bf16).astype(f32)

    class FFN:
        def __init__(self, r, h):
            self.r = r
            self.n = h.shape[0]
            h = h.astype(bf16).astype(f32)
            self.hn = _ln(h).astype(bf16)
            self.acc = h
            self.a = {}

        def gu(self, k):
            g = mm(self.hn, wg_v[:, k * FC:(k + 1) * FC])
            u = mm(self.hn, wu_v[:, k * FC:(k + 1) * FC])
            self.a[k] = (g * jax.nn.sigmoid(g) * u).astype(bf16)

        def down(self, k):
            self.acc = self.acc + mm(self.a.pop(k), wd_v[k * FC:(k + 1) * FC, :])

        def finish(self):
            out_v[pl.ds(self.r, self.n), :] = self.acc.astype(bf16)

    P = functools.partial
    MID = len(order) // 2

    def super_step(j, carry):
        @pl.when(j == 1)
        def _():
            out_copy(1).start()

        @pl.when(j >= 2)
        def _():
            out_copy(j).start()
        mem = mem_v[...]
        xr = pl.multiple_of(PRO + SUB * RIDE * j, 32)
        xns = [xn_v[pl.ds(pl.multiple_of(xr + k * RIDE, 8), RIDE), :] for k in range(SUB)]
        xr_next = pl.multiple_of(PRO + SUB * RIDE * jnp.minimum(j + 1, NSUP - 1), 32)

        def seg(k, mem, extra):
            s = SUB * j + k
            a, mem = segment(s, xns[k], mem, extra)
            return x_v[pl.ds(pl.multiple_of(s * SEG, SEG), SEG), :].astype(f32) + a, mem

        fa = FFN(pl.multiple_of(jnp.maximum(SUB * j - 1, 0) * SEG, SEG), h_v[...])
        h0, mem = seg(0, mem, {MID: [P(ln_rows, xr_next, SUB * RIDE)]})
        h1, mem = seg(1, mem, {0: [P(fa.gu, 0)]})
        h2, mem = seg(2, mem, {0: [P(fa.gu, 1)]})
        fb = FFN(pl.multiple_of(SUB * j * SEG, SEG), jnp.concatenate([h0, h1, h2], axis=0))
        h3, mem = seg(3, mem, {0: [P(fa.down, 0), P(fa.down, 1), fa.finish], 9: [P(fb.gu, 0)], 20: [P(fb.gu, 1)],
                               MID: [P(fb.down, 0)], MID + 12: [P(fb.down, 1), fb.finish]})
        h_v[...] = h3
        mem_v[...] = mem
        return carry

    lax.fori_loop(0, NSUP, super_step, 0)

    out_copy(NSUP).start()
    ffn = FFN(S - SEG, h_v[...])
    ffn.gu(0)
    ffn.gu(1)
    ffn.down(0)
    ffn.down(1)
    ffn.finish()
    out_copy(NSUP + 1).start()
    for j in range(1, NSUP + 2):
        out_copy(j).wait()


@jax.jit
def pallas_sequential_preLN__memory_aug_recurrent_mem_tr__swiglu_ffn__prompt_kernel(
        A_x, A_mem0, A_Wq, A_Wk, A_Wv, A_Wo, A_seg_len, B_x, B_w_gate, B_w_up, B_w_down):
    del A_seg_len, B_x
    x = A_x.reshape(S, D)
    mem0 = A_mem0.reshape(M, D)
    wqt = jnp.transpose(A_Wq, (1, 2, 0)).reshape(HD, D)
    wkt = jnp.transpose(A_Wk, (1, 2, 0)).reshape(HD, D)
    wvt = jnp.transpose(A_Wv, (1, 2, 0)).reshape(HD, D)
    wo = A_Wo.reshape(HD, D)
    any_spec = pl.BlockSpec(memory_space=pl.ANY)
    out = pl.pallas_call(
        _kernel,
        out_shape=jax.ShapeDtypeStruct((S, D), bf16),
        in_specs=[any_spec] * 9,
        out_specs=any_spec,
        scratch_shapes=[
            pltpu.VMEM((S, D), bf16),
            pltpu.VMEM((S, D), bf16),
            pltpu.VMEM((NBUF * CH + HD, D), bf16),
            pltpu.VMEM((D // 2, 3 * HD), u32),
            pltpu.VMEM((HD // 2, D), u32),
            pltpu.VMEM((D, F), bf16),
            pltpu.VMEM((D, F), bf16),
            pltpu.VMEM((F, D), bf16),
            pltpu.VMEM((RING, 3 * HD), bf16),
            pltpu.VMEM((SEG, D), f32),
            pltpu.VMEM((M, D), f32),
            pltpu.VMEM((M, D), bf16),
            pltpu.VMEM((S, D), bf16),
            pltpu.SemaphoreType.DMA((3,)),
            pltpu.SemaphoreType.DMA((NBUF,)),
            pltpu.SemaphoreType.DMA((NFIRST,)),
            pltpu.SemaphoreType.DMA((NWP,)),
            pltpu.SemaphoreType.DMA((3,)),
            pltpu.SemaphoreType.DMA((NSUP + 2,)),
        ],
        compiler_params=pltpu.CompilerParams(vmem_limit_bytes=110 * 1024 * 1024, disable_bounds_checks=True, disable_semaphore_checks=True),
    )(x, mem0, wqt, wkt, wvt, wo, B_w_gate, B_w_up, B_w_down)
    return out.reshape(1, S, D)
```
